```python
import jax
import jax.numpy as jnp

def _softmax(x, axis=-1):
    return jax.nn.softmax(x, axis=axis)
def _gelu(x):
    return jax.nn.gelu(x, approximate=True)
def _silu(x):
    return jax.nn.silu(x)
def _sigmoid(x):
    return jax.nn.sigmoid(x)
def _layernorm(x, axis=-1, eps=1e-5):
    m = jnp.mean(x, axis=axis, keepdims=True)
    v = jnp.var(x, axis=axis, keepdims=True)
    return (x - m) / jnp.sqrt(v + eps)
def _scatter_add(tgt, idx, src, axis=0):
    return tgt.at[idx].add(src)
def _segment_sum(src, seg, n):
    return jax.ops.segment_sum(src, seg, n)
class _Rng:
    def __init__(self, key):
        self._k = key
    def _next(self):
        self._k, sub = jax.random.split(self._k)
        return sub
    def normal(self, shape):
        return jax.random.normal(self._next(), shape, dtype=jnp.bfloat16)
    def randint(self, lo, hi, shape):
        return jax.random.randint(self._next(), shape, lo, hi, dtype=jnp.int32)
    def uniform(self, shape, lo=0.0, hi=1.0):
        return jax.random.uniform(self._next(), shape, jnp.bfloat16, lo, hi)
    def permutation(self, n):
        return jax.random.permutation(self._next(), n)


kernel_name = 'interleave_layers__sliding_block_cached__glu_gated_glu__decode'

def setup_inputs():
    _rng = _Rng(jax.random.key(int.from_bytes(__import__("os").urandom(4), "little")))
    _w = (lambda a: (lambda t: t.astype(jnp.bfloat16) if jnp.issubdtype(t.dtype, jnp.floating) else t)(jnp.asarray(a)))
    def _A_setup():
        B, Sq, D = 1, 1, 640
        Hq, Hkv, Sk, Dh = 32, 32, 32768, 192
        assert Hq % Hkv == 0, (Hq, Hkv)
        return {
            "x": _w((lambda *s: _rng.normal(s) * 0.05)(B, Sq, D)),
            "k_cache": _w((lambda *s: _rng.normal(s) * 0.05)(B, Hkv, Sk, Dh)),
            "v_cache": _w((lambda *s: _rng.normal(s) * 0.05)(B, Hkv, Sk, Dh)),
            "wq": _w((lambda *s: _rng.normal(s) * 0.05)(D, Hq * Dh) * (D ** -0.5)),
            "wo": _w((lambda *s: _rng.normal(s) * 0.05)(Hq * Dh, D) * ((Hq * Dh) ** -0.5)),
        }
    _A_in = _A_setup()

    def _B_setup():
        B, S, D, F = 1, 1, 640, 1536
        return {
            "x": _w((lambda *s: _rng.normal(s) * 0.05)(B, S, D)),
            "w_gate": _w((lambda *s: _rng.normal(s) * 0.05)(D, F)),
            "w_up": _w((lambda *s: _rng.normal(s) * 0.05)(D, F)),
            "w_down": _w((lambda *s: _rng.normal(s) * 0.05)(F, D)),
        }
    _B_in = _B_setup()

    return {
        "A_x": _A_in["x"],
        "A_k_cache": _A_in["k_cache"],
        "A_v_cache": _A_in["v_cache"],
        "A_wq": _A_in["wq"],
        "A_wo": _A_in["wo"],
        "B_x": _B_in["x"],
        "B_w_gate": _B_in["w_gate"],
        "B_w_up": _B_in["w_up"],
        "B_w_down": _B_in["w_down"],
    }

def reference(A_x, A_k_cache, A_v_cache, A_wq, A_wo, B_x, B_w_gate, B_w_up, B_w_down):
    def _A_ref(x, k_cache, v_cache, wq, wo):
        B, Sq, D = x.shape
        Hq, Dh = 32, 192
        Hkv, Sk = k_cache.shape[1], k_cache.shape[2]
        W = min(4096, max(256, Sk // 4))
        rep = Hq // Hkv
        q = (lambda x, *d: x.transpose(*d))((x @ wq).reshape(B, Sq, Hq, Dh), 0, 2, 1, 3)
        k = jnp.repeat(k_cache[:, :, Sk - W:, :], rep, axis=1)
        v = jnp.repeat(v_cache[:, :, Sk - W:, :], rep, axis=1)
        scores = jnp.einsum("bhqd,bhkd->bhqk", q, k) * (Dh ** -0.5)
        p = _softmax(scores, axis=-1)
        o = jnp.einsum("bhqk,bhkd->bhqd", p, v)
        return (lambda x, *d: x.transpose(*d))(o, 0, 2, 1, 3).reshape(B, Sq, Hq * Dh) @ wo

    def _B_ref(x, w_gate, w_up, w_down):
        g = jnp.einsum("bsd,df->bsf", x, w_gate)
        u = jnp.einsum("bsd,df->bsf", x, w_up)
        h = _sigmoid(g) * u
        return jnp.einsum("bsf,fd->bsd", h, w_down)

    x = A_x
    x = x + _A_ref(_layernorm(x, axis=-1), A_k_cache, A_v_cache, A_wq, A_wo)
    x = x + _B_ref(_layernorm(x, axis=-1), B_w_gate, B_w_up, B_w_down)
    x = x + _A_ref(_layernorm(x, axis=-1), A_k_cache, A_v_cache, A_wq, A_wo)
    x = x + _B_ref(_layernorm(x, axis=-1), B_w_gate, B_w_up, B_w_down)
    return x
```

```python
import jax
import jax.numpy as jnp
from jax import lax
import jax.experimental.pallas as pl
import jax.experimental.pallas.tpu as pltpu

H, DH, SK, D, F = 32, 192, 32768, 640, 1536
W = min(4096, max(256, SK // 4))
NP = H // 2
RT = DH // 8
WR = W // 128 * 8
SR = SK // 128 * 8
EPS = 1e-5
bf16, f32, u32 = jnp.bfloat16, jnp.float32, jnp.uint32


def _raw(a):
    r, c = a.shape
    return a.reshape(r // 8, 8, c // 128, 128).transpose(0, 2, 1, 3).reshape(r // 8, c // 128 * 8, 128)


def _ln(x):
    m = jnp.sum(x, axis=-1, keepdims=True) * (1.0 / D)
    d = x - m
    v = jnp.sum(d * d, axis=-1, keepdims=True) * (1.0 / D)
    return (d * lax.rsqrt(v + EPS)).astype(bf16)


def _b(x):
    return pltpu.bitcast(x, bf16)


def _dot(a, b):
    return jnp.dot(a, b, preferred_element_type=f32)


def make(chunk=8, npass=2, look=2, wd_chunks=3, dma=True):
    def kernel(x_hbm, k_hbm, v_hbm, wq_hbm, wo_hbm, wg_hbm, wu_hbm, wd_hbm, o_ref,
               xb, kb, vb, wq, wo, wg, wu, wd, xn_s, q_s, p_s, acc_s, y_s,
               sem_x, sem_q, sem_k, sem_v, sem_o, sem_m):
        k_hbm, v_hbm, wq_hbm, wo_hbm = (r.bitcast(u32) for r in (k_hbm, v_hbm, wq_hbm, wo_hbm))

        def cp_x():
            return pltpu.make_async_copy(x_hbm, xb, sem_x.at[0])

        def cp_q(t):
            return pltpu.make_async_copy(wq_hbm.at[:, pl.ds(128 * t, 128)], wq.at[t], sem_q.at[0])

        def cp_kv(hbm, buf, sem, p):
            rows = pl.ds(p * (2 * RT), 2 * RT)
            return pltpu.make_async_copy(hbm.at[rows, pl.ds((SR - WR) // 2, WR // 2)], buf.at[rows], sem.at[p])

        def cp_o(p, c):
            r0 = pl.multiple_of(p * DH, 64)
            return pltpu.make_async_copy(
                wo_hbm.at[pl.ds(r0, DH), pl.ds(128 * c, 128)], wo.at[p * 5 + c], sem_o.at[p])

        fr = F // wd_chunks

        def cp_m(j):
            if j == 0:
                return pltpu.make_async_copy(wg_hbm, wg, sem_m.at[0])
            if j == 1:
                return pltpu.make_async_copy(wu_hbm, wu, sem_m.at[1])
            rows = pl.ds((j - 2) * fr, fr)
            return pltpu.make_async_copy(wd_hbm.at[rows], wd.at[rows], sem_m.at[j])

        def start_step(s):
            cp_kv(v_hbm, vb, sem_v, s).start()
            for c in range(5):
                cp_o(s, c).start()

        if dma:
            cp_x().start()
            for t in range(3 * NP):
                cp_q(t).start()
            cp_kv(k_hbm, kb, sem_k, 0).start()
            for s in range(look):
                cp_kv(k_hbm, kb, sem_k, s + 1).start()
                start_step(s)
            cp_x().wait()
        x0 = jnp.broadcast_to(xb[...].astype(f32), (8, D))

        def stage_a(p, slot):
            w = jnp.concatenate([_b(wq[3 * p + t]) for t in range(3)], axis=1)
            q = _dot(xn_s[...], w)
            q_s[slot] = q

        def stage_b(p, slot):
            lane = lax.broadcasted_iota(jnp.int32, (8, 128), 1)
            sub = lax.broadcasted_iota(jnp.int32, (8, 128), 0)
            diag = ((lane >> 3) & 7) == sub
            base = ((lane >> 6) << 3) + (lane & 7)
            for a in range(2):
                lhs = []
                for kt in range(12):
                    g = 12 * a + kt
                    qt = q_s[slot, :, pl.ds(128 * (g // 8), 128)]
                    e = jnp.take_along_axis(qt, base + 16 * (g % 8), axis=1)
                    lhs.append(jnp.where(diag, e, 0.0).astype(bf16))
                lhs = jnp.concatenate(lhs, axis=1)
                r0 = p * (2 * RT) + a * RT
                rhs = jnp.concatenate(
                    [_b(kb[pl.ds(r0, RT), pl.ds(32 * c, 32), :].reshape(RT * 32, 128)) for c in range(4)],
                    axis=1)
                s = _dot(lhs, rhs) * (DH ** -0.5)
                m = jnp.max(jnp.max(s, axis=1, keepdims=True), axis=0, keepdims=True)
                e = jnp.exp(s - m)
                l = jnp.sum(jnp.sum(e, axis=1, keepdims=True), axis=0, keepdims=True)
                pr = e * (1.0 / l)
                for c in range(4):
                    p_s[slot, pl.ds(32 * a + 8 * c, 8), :] = pr[:, 128 * c:128 * (c + 1)]

        def stage_c(p, slot):
            for a in range(2):
                for r in range(0, RT, chunk):
                    r0 = p * (2 * RT) + a * RT + r
                    acc = None
                    for j in range(WR // 16):
                        v = _b(vb[pl.ds(r0, chunk), pl.ds(8 * j, 8), :]).astype(f32)
                        p0 = jnp.broadcast_to(p_s[slot, pl.ds(32 * a + 2 * j, 1), :], (8, 128))
                        p1 = jnp.broadcast_to(p_s[slot, pl.ds(32 * a + 2 * j + 1, 1), :], (8, 128))
                        t = v[:, :8, :] * p0 + v[:, 8:, :] * p1
                        acc = t if acc is None else acc + t
                    acc_s[slot, pl.ds((a * RT + r) * 8, chunk * 8), :] = acc.reshape(chunk * 8, 128)

        def stage_d(p, slot):
            o = []
            for t in range(3):
                tt = acc_s[slot, pl.ds(128 * t, 128), :].T
                o.append(jnp.broadcast_to(jnp.sum(tt, axis=0, keepdims=True), (8, 128)))
            o = jnp.concatenate(o, axis=1).astype(bf16)
            w = jnp.concatenate([_b(wo[5 * p + c]) for c in range(5)], axis=1)
            return _dot(o, w)

        def layer(ps, x):
            first = ps == 0
            xn_s[...] = _ln(x)

            if dma:
                @pl.when(first)
                def _():
                    for t in range(3 * NP):
                        cp_q(t).wait()
                    cp_kv(k_hbm, kb, sem_k, 0).wait()

            stage_a(0, 0)
            stage_a(1, 1)
            stage_b(0, 0)
            acc_s[1] = jnp.zeros(acc_s.shape[1:], f32)
            y_s[...] = jnp.zeros(y_s.shape, f32)

            def step(i, carry):
                if dma:
                    @pl.when(first)
                    def _():
                        @pl.when(i + look + 1 < NP)
                        def _():
                            cp_kv(k_hbm, kb, sem_k, i + look + 1).start()

                        @pl.when(i + look < NP)
                        def _():
                            start_step(i + look)

                        @pl.when(i + look == NP)
                        def _():
                            for j in range(2 + wd_chunks):
                                cp_m(j).start()

                        @pl.when(i + 1 < NP)
                        def _():
                            cp_kv(k_hbm, kb, sem_k, i + 1).wait()

                        cp_kv(v_hbm, vb, sem_v, i).wait()
                        for c in range(5):
                            cp_o(i, c).wait()

                cur = i & 1
                nxt = 1 - cur
                stage_b(jnp.minimum(i + 1, NP - 1), nxt)
                y = stage_d(jnp.maximum(i - 1, 0), nxt)
                y_s[...] += jnp.where(i > 0, y, 0.0)
                stage_a(jnp.minimum(i + 2, NP - 1), cur)
                stage_c(i, cur)
                return carry

            lax.fori_loop(0, NP, step, 0)
            x = x + (y_s[...] + stage_d(NP - 1, (NP - 1) & 1))

            xn = _ln(x)
            if dma:
                @pl.when(first)
                def _():
                    cp_m(0).wait()
                    cp_m(1).wait()
            g = _dot(xn, wg[...])
            u = _dot(xn, wu[...])
            h = ((1.0 / (1.0 + jnp.exp(-g))) * u).astype(bf16)
            for j in range(wd_chunks):
                if dma:
                    @pl.when(first)
                    def _():
                        cp_m(2 + j).wait()
                x = x + _dot(h[:, j * fr:(j + 1) * fr], wd[pl.ds(j * fr, fr), :])
            return x

        x = lax.fori_loop(0, npass, layer, x0)
        o_ref[...] = x[:1].astype(o_ref.dtype)

    @jax.jit
    def fn(A_x, A_k_cache, A_v_cache, A_wq, A_wo, B_x, B_w_gate, B_w_up, B_w_down):
        del B_x
        kt = _raw(jnp.swapaxes(A_k_cache, 2, 3).reshape(H * DH, SK))
        vt = _raw(jnp.swapaxes(A_v_cache, 2, 3).reshape(H * DH, SK))
        hbm = pl.BlockSpec(memory_space=pltpu.HBM)
        out = pl.pallas_call(
            kernel,
            out_shape=jax.ShapeDtypeStruct((1, D), bf16),
            in_specs=[hbm] * 8,
            out_specs=pl.BlockSpec(memory_space=pltpu.VMEM),
            scratch_shapes=[
                pltpu.VMEM((1, D), bf16),
                pltpu.VMEM((H * RT, WR // 2, 128), u32),
                pltpu.VMEM((H * RT, WR // 2, 128), u32),
                pltpu.VMEM((3 * NP, D // 2, 128), u32),
                pltpu.VMEM((5 * NP, DH, 128), u32),
                pltpu.VMEM((D, F), bf16),
                pltpu.VMEM((D, F), bf16),
                pltpu.VMEM((F, D), bf16),
                pltpu.VMEM((8, D), bf16),
                pltpu.VMEM((2, 8, 2 * DH), f32),
                pltpu.VMEM((2, 64, 128), f32),
                pltpu.VMEM((2, 2 * DH, 128), f32),
                pltpu.VMEM((8, D), f32),
                pltpu.SemaphoreType.DMA((1,)),
                pltpu.SemaphoreType.DMA((1,)),
                pltpu.SemaphoreType.DMA((NP,)),
                pltpu.SemaphoreType.DMA((NP,)),
                pltpu.SemaphoreType.DMA((NP,)),
                pltpu.SemaphoreType.DMA((2 + wd_chunks,)),
            ],
            compiler_params=pltpu.CompilerParams(vmem_limit_bytes=127 * 1024 * 1024),
        )(A_x.reshape(1, D), kt, vt, A_wq, A_wo, B_w_gate, B_w_up, B_w_down)
        return out.reshape(1, 1, D)

    return fn


_fn = make()


@jax.jit
def pallas_interleave_layers__sliding_block_cached__glu_gated_glu__decode_kernel(
    A_x, A_k_cache, A_v_cache, A_wq, A_wo, B_x, B_w_gate, B_w_up, B_w_down
):
    return _fn(A_x, A_k_cache, A_v_cache, A_wq, A_wo, B_x, B_w_gate, B_w_up, B_w_down)
```

```python
import jax
import jax.numpy as jnp
from jax import lax
import jax.experimental.pallas as pl
import jax.experimental.pallas.tpu as pltpu

H, DH, SK, D, F = 32, 192, 32768, 640, 1536
W = min(4096, max(256, SK // 4))
NP = H // 2
RT = DH // 8
NT = W // 128
NZ = 16
EPS = 1e-5
bf16, f32, u32 = jnp.bfloat16, jnp.float32, jnp.uint32


def _raw(a):
    r, c = a.shape
    return a.reshape(r // 8, 8, c // 128, 128).transpose(0, 2, 1, 3).reshape(r // 8, c // 128 * 8, 128)


def _ln(x):
    m = jnp.sum(x, axis=-1, keepdims=True) * (1.0 / D)
    d = x - m
    v = jnp.sum(d * d, axis=-1, keepdims=True) * (1.0 / D)
    return d * lax.rsqrt(v + EPS)


def _b(x):
    return pltpu.bitcast(x, bf16)


def _dot(a, b):
    return lax.dot_general(a, b, (((1,), (0,)), ((), ())), preferred_element_type=f32)


def _iota(axis):
    return lax.broadcasted_iota(jnp.int32, (8, 128), axis)


def _run(*gens):
    for g in gens:
        for _ in g:
            pass


def _chain(*gens):
    for g in gens:
        yield from g


class _Pace:
    def __init__(self, m_ref=None, v_ref=None, z_ref=None):
        self.refs, self.z_ref = (m_ref, v_ref), z_ref
        self.now, self.due, self.slot = 0, ({}, {}), [0, 0]

    def before_mxu(self, key, val, delay):
        self.due[0][key, self.now] = (self.now + delay, val)

    def before_vpu(self, key, val, delay):
        self.due[1][key, self.now] = (self.now + delay, val)

    def tick(self, mxu=True):
        self.now += 1
        for w in (0, 1) if mxu else (1,):
            ref, due = self.refs[w], self.due[w]
            for key in [k for k, (t, _) in due.items() if t <= self.now]:
                self.slot[w] = (self.slot[w] + 1) % NZ
                ref(self.slot[w], due.pop(key)[1])

    def zero(self):
        if self.z_ref is None:
            return jnp.zeros((8, 128), f32)
        return self.z_ref[0]


def make(chunk=4, npass=2, look=2, wd_chunks=3, dma=True, mfrac=0.85, order="a0x1yd", tree=True,
         k_acc=1, k_fold=8, dk_fold=5, k_sm=14, k_sm1=12, defer=True, tail=True, every=1, gm='z', gv='p', k_q=8, nit=NP, k_m=4, last_free=False, flags=None):
    def kernel(x_hbm, k_hbm, v_hbm, wq_hbm, wo_hbm, wg_hbm, wu_hbm, wd_hbm, o_ref,
               xb, kb, vb, wq, wo, wg, wu, wd, xn_s, q_s, s_s, p_s, pb_s, z_s, acc_s, y_s,
               sem_x, sem_q, sem_k, sem_v, sem_o, sem_m):
        k_hbm, v_hbm, wq_hbm, wo_hbm = (r.bitcast(u32) for r in (k_hbm, v_hbm, wq_hbm, wo_hbm))

        def cp_x():
            return pltpu.make_async_copy(x_hbm, xb, sem_x.at[0])

        def cp_q(t):
            return pltpu.make_async_copy(wq_hbm.at[:, pl.ds(128 * t, 128)], wq.at[t], sem_q.at[0])

        def cp_kv(hbm, buf, sem, p):
            rows = pl.ds(p * (2 * RT), 2 * RT)
            return pltpu.make_async_copy(
                hbm.at[rows, pl.ds((SK - W) // 32, W // 32)], buf.at[rows], sem.at[p])

        def cp_o(p, c):
            r0 = pl.multiple_of(p * DH, 64)
            return pltpu.make_async_copy(
                wo_hbm.at[pl.ds(r0, DH), pl.ds(128 * c, 128)], wo.at[p * 5 + c], sem_o.at[p])

        fr = F // wd_chunks

        def cp_m(j):
            if j == 0:
                return pltpu.make_async_copy(wg_hbm, wg, sem_m.at[0])
            if j == 1:
                return pltpu.make_async_copy(wu_hbm, wu, sem_m.at[1])
            rows = pl.ds((j - 2) * fr, fr)
            return pltpu.make_async_copy(wd_hbm.at[rows], wd.at[rows], sem_m.at[j])

        def start_step(s):
            cp_kv(v_hbm, vb, sem_v, s).start()
            for c in range(5):
                cp_o(s, c).start()

        if dma:
            cp_x().start()
            for t in range(3 * NP):
                cp_q(t).start()
            cp_kv(k_hbm, kb, sem_k, 0).start()
            for s in range(look):
                cp_kv(k_hbm, kb, sem_k, s + 1).start()
                start_step(s)
            cp_x().wait()
        z_s[0] = jnp.zeros((8, 128), f32)
        x0 = jnp.broadcast_to(xb[...].astype(f32), (8, D))

        def stage_a(p, pace, out):
            q = None
            for k in range(5):
                w = jnp.concatenate([_b(wq[3 * p + t, pl.ds(64 * k, 64), :]) for t in range(3)], axis=1)
                t = _dot(xn_s[:, pl.ds(128 * k, 128)] + pace.zero(), w)
                q = t if q is None else q + t
                pace.before_vpu(0, q[:, :128], k_m)
                yield
            out.append(q)

        def spread(q, a, pace):
            lane = _iota(1)
            for g in range(12 * a, 12 * a + 12):
                qt = q[:, 128 * (g // 8):128 * (g // 8 + 1)]
                e = jnp.take_along_axis(qt, ((lane >> 6) << 3) + (lane & 7) + 16 * (g % 8), axis=1)
                q_s[g] = e
                if g % 4 == 3:
                    pace.before_vpu(("q", g), e, k_q)

        def stage_b(p, a, pace, done=None):
            diag = ((_iota(1) >> 3) & 7) == _iota(0)
            s = None
            for kt in range(12):
                lhs = jnp.where(diag, q_s[12 * a + kt], pace.zero())
                r0 = p * (2 * RT) + a * RT + 2 * kt
                rhs = jnp.concatenate(
                    [_b(kb[pl.ds(r0, 2), pl.ds(32 * c, 32), :].reshape(64, 128)) for c in range(4)],
                    axis=1)
                t = _dot(lhs, rhs)
                s = t if s is None else s + t
                pace.before_vpu(0, s[:, :128], k_m)
                yield
            if a == 1 and defer:
                s_s[...] = s
            else:
                softmax(s, a, pace, k_sm, done)

        def softmax(s, a, pace, k, done=None):
            s = s * (DH ** -0.5)
            m = jnp.max(jnp.max(s, axis=1, keepdims=True), axis=0, keepdims=True)
            e = jnp.exp(s - m)
            l = jnp.sum(jnp.sum(e, axis=1, keepdims=True), axis=0, keepdims=True)
            assert done is None or a in done
            pr = e * (1.0 / l)
            p_s[a] = pr
            pace.before_vpu(("sm", a), pr[:, :128], k)

        def stage_c(p, pace, done):
            for a in range(2):
                pr = p_s[a]
                done.add(a)
                for r in range(0, RT, chunk):
                    r0 = p * (2 * RT) + a * RT + r
                    acc = [None] * chunk
                    for j in range(NT // 2):
                        pp = []
                        for t in (2 * j, 2 * j + 1):
                            if r == 0:
                                pb_s[NT * a + t] = jnp.broadcast_to(
                                    pr[t % 8:t % 8 + 1, 128 * (t // 8):128 * (t // 8 + 1)], (8, 128))
                            pp.append(pb_s[NT * a + t])
                        p0, p1 = pp
                        for n in range(chunk):
                            v = _b(vb[r0 + n, pl.ds(8 * j, 8), :]).astype(f32)
                            if acc[n] is None:
                                acc[n] = v[:8] * p0 + v[8:] * p1
                            elif tree:
                                acc[n] = acc[n] + (v[:8] * p0 + v[8:] * p1)
                            else:
                                acc[n] = (acc[n] + v[:8] * p0) + v[8:] * p1
                            if j + 1 < NT // 2 or not last_free:
                                pace.before_mxu((a, r, n), acc[n], k_acc)
                            yield
                    for n in range(chunk):
                        acc_s[a * RT + r + n] = acc[n]

        def stage_d1():
            tiles = []
            for rt in range(2 * RT):
                col = jnp.broadcast_to(jnp.sum(acc_s[rt], axis=1, keepdims=True), (8, 128))
                if rt % 16 == 0:
                    tiles.append(col)
                else:
                    tiles[-1] = jnp.where((_iota(1) >> 3) == rt % 16, col, tiles[-1])
            return tiles

        def stage_d2(p, tiles, pace, put):
            y = None
            for t in range(3):
                w = jnp.concatenate([_b(wo[5 * p + c, pl.ds(64 * t, 64), :]) for c in range(5)], axis=1)
                o = jnp.where((_iota(1) & 7) == _iota(0), tiles[t], pace.zero())
                z = _dot(o, w)
                y = z if y is None else y + z
                pace.before_vpu(0, y[:, :128], k_m)
                yield
            put(y)

        def call(f):
            f()
            return
            yield

        def layer(ps, x):
            first = ps == 0
            xn_s[...] = _ln(x)

            if dma:
                @pl.when(first)
                def _():
                    for t in range(3 * NP):
                        cp_q(t).wait()
                    cp_kv(k_hbm, kb, sem_k, 0).wait()

            free = _Pace()
            q = []
            _run(stage_a(0, free, q))
            spread(q[0], 0, free)
            spread(q[0], 1, free)
            _run(stage_a(1, free, q), stage_b(0, 0, free), stage_b(0, 1, free))
            spread(q[1], 0, free)
            spread(q[1], 1, free)
            acc_s[...] = jnp.zeros(acc_s.shape, f32)
            y_s[...] = jnp.zeros(y_s.shape, f32)

            def step(i, carry):
                if dma:
                    @pl.loop(ps, 1)
                    def _(_):
                        @pl.when(i + look + 1 < NP)
                        def _():
                            cp_kv(k_hbm, kb, sem_k, i + look + 1).start()

                        @pl.when(i + look < NP)
                        def _():
                            start_step(i + look)

                        @pl.when(i + look == NP)
                        def _():
                            for j in range(2 + wd_chunks):
                                cp_m(j).start()

                        @pl.when(i + 1 < NP)
                        def _():
                            cp_kv(k_hbm, kb, sem_k, i + 1).wait()

                        cp_kv(v_hbm, vb, sem_v, i).wait()
                        for c in range(5):
                            cp_o(i, c).wait()

                def fin(y):
                    y_s[...] += jnp.where(i > 0, y, 0.0)

                done = set()
                def small(ref):
                    def f(slot, val):
                        ref[ref.shape[0] - 1 - slot - (i >> 8)] = val
                    return f

                def big(*refs):
                    def f(slot, val):
                        for ref in refs:
                            ref[ref.shape[0] - 1 - (i >> 8), pl.ds(8 * slot, 8), :] = pltpu.bitcast(val, u32)
                    return f

                pace = _Pace(small(z_s) if gm == "z" else big(kb, wq, wo),
                             small(pb_s) if gv == "p" else big(vb), z_s if gm == "z" else None)
                q = []
                if defer:
                    softmax(s_s[...], 1, pace, k_sm1)
                tiles = stage_d1()
                for t in range(3):
                    pace.before_vpu(("o", t), tiles[t], k_fold + dk_fold * t)
                pn = jnp.minimum(i + 1, NP - 1)
                st = {"0": stage_b(pn, 0, pace, done), "1": stage_b(pn, 1, pace, done),
                      "d": stage_d2(jnp.maximum(i - 1, 0), tiles, pace, fin),
                      "a": stage_a(jnp.minimum(i + 2, NP - 1), pace, q),
                      "x": call(lambda: spread(q[0], 0, pace)),
                      "y": call(lambda: spread(q[0], 1, pace))}
                mxu = _chain(*[st[k] for k in order])
                vpu = stage_c(i, pace, done)
                per = int(768 * mfrac / 32)
                for e in range(-(-768 // per)):
                    next(mxu, None)
                    for _ in range(per):
                        next(vpu, None)
                    if (e < 31 or tail) and e % every == every - 1:
                        pace.tick(e < 31)
                    else:
                        pace.now += 1
                _run(mxu, vpu)
                return carry

            lax.fori_loop(0, nit, step, 0)

            def fin(y):
                y_s[...] += y
            _run(stage_d2(NP - 1, stage_d1(), free, fin))
            x = x + jnp.sum(y_s[...], axis=0, keepdims=True)

            xn = _ln(x)
            if dma:
                @pl.when(first)
                def _():
                    cp_m(0).wait()
                    cp_m(1).wait()
            g = _dot(xn, wg[...])
            u = _dot(xn, wu[...])
            h = (1.0 / (1.0 + jnp.exp(-g))) * u
            for j in range(wd_chunks):
                if dma:
                    @pl.when(first)
                    def _():
                        cp_m(2 + j).wait()
                x = x + _dot(h[:, j * fr:(j + 1) * fr], wd[pl.ds(j * fr, fr), :])
            return x

        x = lax.fori_loop(0, npass, layer, x0)
        o_ref[...] = x[:1].astype(o_ref.dtype)

    @jax.jit
    def fn(A_x, A_k_cache, A_v_cache, A_wq, A_wo, B_x, B_w_gate, B_w_up, B_w_down):
        del B_x
        kt = _raw(jnp.swapaxes(A_k_cache, 2, 3).reshape(H * DH, SK))
        vt = _raw(jnp.swapaxes(A_v_cache, 2, 3).reshape(H * DH, SK))
        hbm = pl.BlockSpec(memory_space=pltpu.HBM)
        out = pl.pallas_call(
            kernel,
            out_shape=jax.ShapeDtypeStruct((1, D), bf16),
            in_specs=[hbm] * 8,
            out_specs=pl.BlockSpec(memory_space=pltpu.VMEM),
            scratch_shapes=[
                pltpu.VMEM((1, D), bf16),
                pltpu.VMEM((H * RT + 1, W // 32, 128), u32),
                pltpu.VMEM((H * RT + 1, W // 32, 128), u32),
                pltpu.VMEM((3 * NP + 1, D // 2, 128), u32),
                pltpu.VMEM((5 * NP + 1, DH, 128), u32),
                pltpu.VMEM((D, F), bf16),
                pltpu.VMEM((D, F), bf16),
                pltpu.VMEM((F, D), bf16),
                pltpu.VMEM((8, D), f32),
                pltpu.VMEM((24, 8, 128), f32),
                pltpu.VMEM((8, 512), f32),
                pltpu.VMEM((2, 8, 512), f32),
                pltpu.VMEM((2 * NT + NZ, 8, 128), f32),
                pltpu.VMEM((NZ + 1, 8, 128), f32),
                pltpu.VMEM((2 * RT, 8, 128), f32),
                pltpu.VMEM((8, D), f32),
                pltpu.SemaphoreType.DMA((1,)),
                pltpu.SemaphoreType.DMA((1,)),
                pltpu.SemaphoreType.DMA((NP,)),
                pltpu.SemaphoreType.DMA((NP,)),
                pltpu.SemaphoreType.DMA((NP,)),
                pltpu.SemaphoreType.DMA((2 + wd_chunks,)),
            ],
            compiler_params=pltpu.CompilerParams(vmem_limit_bytes=127 * 1024 * 1024, disable_semaphore_checks=True, flags=flags),
        )(A_x.reshape(1, D), kt, vt, A_wq, A_wo, B_w_gate, B_w_up, B_w_down)
        return out.reshape(1, 1, D)

    return fn


_fn = make(**dict(gm='z',gv='v',k_m=5,k_acc=2,mfrac=0.88,chunk=4,k_q=12,k_sm=20,k_sm1=60,k_fold=10,dk_fold=3,tree=False,order='a0xd1y'))


@jax.jit
def pallas_interleave_layers__sliding_block_cached__glu_gated_glu__decode_kernel(
    A_x, A_k_cache, A_v_cache, A_wq, A_wo, B_x, B_w_gate, B_w_up, B_w_down
):
    return _fn(A_x, A_k_cache, A_v_cache, A_wq, A_wo, B_x, B_w_gate, B_w_up, B_w_down)
```

```python
import jax
import jax.numpy as jnp
from jax import lax
import jax.experimental.pallas as pl
import jax.experimental.pallas.tpu as pltpu

H, DH, SK, D, F = 32, 192, 32768, 640, 1536
W = min(4096, max(256, SK // 4))
NP = H // 2
RT = DH // 8
NT = W // 128
NZ = 16
EPS = 1e-5
bf16, f32, u32 = jnp.bfloat16, jnp.float32, jnp.uint32


def _raw(a):
    r, c = a.shape
    return a.reshape(r // 8, 8, c // 128, 128).transpose(0, 2, 1, 3).reshape(r // 8, c // 128 * 8, 128)


def _ln(x):
    d = x - jnp.sum(x, axis=-1, keepdims=True) * (1.0 / D)
    v = jnp.sum(d * d, axis=-1, keepdims=True) * (1.0 / D)
    return d, jnp.broadcast_to(lax.rsqrt(v + EPS), (8, 128))


def _wide(x, n):
    return jnp.concatenate([x] * n, axis=1)


def _b(x):
    return pltpu.bitcast(x, bf16)


def _dot(a, b):
    return lax.dot_general(a, b, (((1,), (0,)), ((), ())), preferred_element_type=f32)


def _iota(axis):
    return lax.broadcasted_iota(jnp.int32, (8, 128), axis)


def _run(*gens):
    for g in gens:
        for _ in g:
            pass


def _chain(*gens):
    for g in gens:
        yield from g


def _call(f):
    f()
    return
    yield


class _Pace:
    def __init__(self, to_mxu=None, to_vpu=None, z_ref=None):
        self.put, self.z_ref = (to_mxu, to_vpu), z_ref
        self.now, self.due, self.slot = 0, ({}, {}), [0, 0]

    def before_mxu(self, key, val, delay):
        self.due[0][key, self.now] = (self.now + delay, val)

    def before_vpu(self, key, val, delay):
        self.due[1][key, self.now] = (self.now + delay, val)

    def tick(self, mxu):
        self.now += 1
        for w in (0, 1) if mxu else (1,):
            due = self.due[w]
            for key in [k for k, (t, _) in due.items() if t <= self.now]:
                self.slot[w] = (self.slot[w] + 1) % NZ
                self.put[w](self.slot[w], due.pop(key)[1])

    def zero(self):
        if self.z_ref is None:
            return jnp.zeros((8, 128), f32)
        return self.z_ref[0, pl.ds(0, 8), :]


def make(chunk=4, npass=2, look=2, dma=True, lag=5, order="a0xd1ye", tree=False,
         k_acc=2, k_fold=10, dk_fold=3, k_sm=20, k_sm1=60, k_q=12, k_m=5, nit=NP, mt=2, fl=256,
         jg=1, sm_first=False, k_self=1, unroll=1, flags=None):
    nv = (NT - mt) // 2

    def kernel(x_hbm, k_hbm, v_hbm, wq_hbm, wo_hbm, wg_hbm, wu_hbm, wd_hbm, o_ref,
               kb, vb, wq, wo, wg, wu, wd, q_s, s_s, p_s, pb_s, acc_s, z_s, e_s, xn_s, y_s, xb,
               sem_x, sem_q, sem_k, sem_v, sem_o, sem_m):
        k_hbm, v_hbm, wq_hbm, wo_hbm = (r.bitcast(u32) for r in (k_hbm, v_hbm, wq_hbm, wo_hbm))

        def cp_x():
            return pltpu.make_async_copy(x_hbm, xb.at[:, pl.ds(0, D)], sem_x.at[0])

        def cp_q(t):
            return pltpu.make_async_copy(wq_hbm.at[:, pl.ds(128 * t, 128)], wq.at[t], sem_q.at[0])

        def cp_kv(hbm, buf, sem, p):
            rows = pl.ds(p * (2 * RT), 2 * RT)
            return pltpu.make_async_copy(
                hbm.at[rows, pl.ds((SK - W) // 32, W // 32)], buf.at[rows], sem.at[p])

        def cp_o(p, c):
            r0 = pl.multiple_of(p * DH, 64)
            return pltpu.make_async_copy(
                wo_hbm.at[pl.ds(r0, DH), pl.ds(128 * c, 128)], wo.at[p * 5 + c], sem_o.at[p])

        def cp_m(j):
            if j < 2:
                return pltpu.make_async_copy((wg_hbm, wu_hbm)[j], (wg, wu)[j], sem_m.at[j])
            rows = pl.ds(0, F - fl) if j == 2 else pl.ds(F - fl, fl)
            return pltpu.make_async_copy(wd_hbm.at[rows], wd.at[rows], sem_m.at[j])

        def start_step(s):
            cp_kv(v_hbm, vb, sem_v, s).start()
            for c in range(5):
                cp_o(s, c).start()

        if dma:
            cp_x().start()
            for t in range(3 * NP):
                cp_q(t).start()
            cp_kv(k_hbm, kb, sem_k, 0).start()
            for s in range(look):
                cp_kv(k_hbm, kb, sem_k, s + 1).start()
                start_step(s)
            cp_x().wait()
        z_s[0, pl.ds(0, 8), :] = jnp.zeros((8, 128), f32)
        x0 = jnp.broadcast_to(xb[:, pl.ds(0, D)].astype(f32), (8, D))

        def stage_a(p, pace, out):
            q = None
            for k in range(5):
                w = jnp.concatenate([_b(wq[3 * p + t, pl.ds(64 * k, 64), :]) for t in range(3)], axis=1)
                t = _dot(xn_s[:, pl.ds(128 * k, 128)] + pace.zero(), w)
                q = t if q is None else q + t
                pace.before_vpu(0, q[:, :128], k_m)
                yield
            out.append(q * _wide(xn_s[:, pl.ds(D, 128)], 3))

        def spread(q, a, pace):
            lane = _iota(1)
            for g in range(12 * a, 12 * a + 12):
                qt = q[:, 128 * (g // 8):128 * (g // 8 + 1)]
                e = jnp.take_along_axis(qt, ((lane >> 6) << 3) + (lane & 7) + 16 * (g % 8), axis=1)
                q_s[g] = e
                if g % 4 == 3:
                    pace.before_vpu(("q", g), e, k_q)

        def stage_b(p, a, pace, seen=None):
            diag = ((_iota(1) >> 3) & 7) == _iota(0)
            s = None
            for kt in range(12):
                lhs = jnp.where(diag, q_s[12 * a + kt], pace.zero())
                r0 = p * (2 * RT) + a * RT + 2 * kt
                rhs = jnp.concatenate(
                    [_b(kb[pl.ds(r0, 2), pl.ds(32 * c, 32), :].reshape(64, 128)) for c in range(4)],
                    axis=1)
                t = _dot(lhs, rhs)
                s = t if s is None else s + t
                pace.before_vpu(0, s[:, :128], k_m)
                yield
            assert seen is None or seen()
            if a == 1:
                s_s[...] = s
            else:
                p_s[...] = softmax(s, a, pace, k_sm)

        def softmax(s, a, pace, k):
            m = jnp.max(jnp.max(s, axis=1, keepdims=True), axis=0, keepdims=True)
            e = jnp.exp(s - m)
            l = jnp.sum(jnp.sum(e, axis=1, keepdims=True), axis=0, keepdims=True)
            pr = e * (1.0 / l)
            pace.before_vpu(("sm", a), pr[:, :128], k)
            return pr

        def row(pr, t):
            return jnp.broadcast_to(pr[t % 8:t % 8 + 1, 128 * (t // 8):128 * (t // 8 + 1)], (8, 128))

        def stage_c(p, prs, pace):
            for a in range(2):
                for r in range(0, RT, chunk):
                    r0 = p * (2 * RT) + a * RT + r
                    acc = [None] * chunk
                    for j0 in range(0, nv, jg):
                        js = range(j0, min(j0 + jg, nv))
                        pp = {}
                        for t in range(2 * js[0], 2 * js[-1] + 2):
                            if r == 0:
                                pb_s[NT * a + t] = row(prs[a], t)
                            pp[t] = pb_s[NT * a + t]
                        for n in range(chunk):
                            for j in js:
                                p0, p1 = pp[2 * j], pp[2 * j + 1]
                                v = _b(vb[r0 + n, pl.ds(8 * j, 8), :]).astype(f32)
                                if acc[n] is None:
                                    acc[n] = v[:8] * p0 + v[8:] * p1
                                elif tree:
                                    acc[n] = acc[n] + (v[:8] * p0 + v[8:] * p1)
                                else:
                                    acc[n] = (acc[n] + v[:8] * p0) + v[8:] * p1
                                pace.before_mxu((a, r, n), acc[n], k_acc)
                                if k_self and pace.now + k_self < k_m:
                                    pace.before_vpu("self", acc[n], k_self)
                                yield
                    for n in range(chunk):
                        acc_s[a * RT + r + n] = acc[n]

        def flip(p):
            for u in range(3):
                for j in range(nv, NT // 2):
                    r0 = p * (2 * RT) + 16 * u
                    v = _b(vb[pl.ds(r0, 16), pl.ds(8 * j, 8), :]).astype(f32)
                    for h in range(2):
                        t = v[:, 8 * h:8 * h + 8, :].reshape(128, 128).T.astype(bf16)
                        vb[pl.ds(r0 + 8 * h, 8), pl.ds(8 * j, 8), :] = pltpu.bitcast(t, u32).reshape(8, 8, 128)

        def stage_e(p, prs, pace):
            o = None
            for t in range(NT - mt, NT):
                lhs = jnp.where(_iota(0) < 4, row(prs[0], t), row(prs[1], t)) + pace.zero()
                w = jnp.concatenate(
                    [_b(vb[pl.ds(p * (2 * RT) + 16 * u + 8 * (t % 2), 8), pl.ds(8 * (t // 2), 8), :]
                        .reshape(64, 128)) for u in range(3)], axis=1)
                z = _dot(lhs, w)
                o = z if o is None else o + z
                pace.before_vpu(0, o[:, :128], k_m)
                yield
            if mt:
                e_s[:, pl.ds(0, 384)] = o

        def stage_d1():
            def merge(lo, n):
                if n == 1:
                    return jnp.broadcast_to(jnp.sum(acc_s[lo], axis=1, keepdims=True), (8, 128))
                n //= 2
                return jnp.where((_iota(1) & (8 * n)) == 0, merge(lo, n), merge(lo + n, n))

            tiles = [merge(16 * t, 16) for t in range(3)]
            return tiles, (e_s[:, pl.ds(0, 384)] if mt else None)

        def stage_d2(p, o, pace, put):
            tiles, extra = o
            y = None
            lane, sub = _iota(1), _iota(0)
            for t in range(3):
                w = jnp.concatenate([_b(wo[5 * p + c, pl.ds(64 * t, 64), :]) for c in range(5)], axis=1)
                lhs = jnp.where((lane & 7) == sub, tiles[t], pace.zero())
                if mt:
                    pick = sub == (0, (lane >> 6) << 2, 4)[t]
                    lhs = lhs + jnp.where(pick, extra[:, 128 * t:128 * (t + 1)], 0.0)
                z = _dot(lhs, w)
                y = z if y is None else y + z
                pace.before_vpu(0, y[:, :128], k_m)
                yield
            put(y)

        def layer(ps, x):
            d, r = _ln(x)
            xn_s[:, pl.ds(0, D)] = d
            xn_s[:, pl.ds(D, 128)] = r * (DH ** -0.5)

            free = _Pace()
            q = []
            _run(stage_a(0, free, q))
            spread(q[0], 0, free)
            spread(q[0], 1, free)
            _run(stage_a(1, free, q), stage_b(0, 0, free), stage_b(0, 1, free))
            spread(q[1], 0, free)
            spread(q[1], 1, free)
            acc_s[...] = jnp.zeros(acc_s.shape, f32)
            e_s[...] = jnp.zeros(e_s.shape, f32)
            y_s[...] = jnp.zeros(y_s.shape, f32)

            def load(i):
                @pl.when(i + look + 1 < NP)
                def _():
                    cp_kv(k_hbm, kb, sem_k, i + look + 1).start()

                @pl.when(i + look < NP)
                def _():
                    start_step(i + look)

                @pl.when(i + look == NP)
                def _():
                    for j in range(4):
                        cp_m(j).start()

                @pl.when(i + 1 < NP)
                def _():
                    cp_kv(k_hbm, kb, sem_k, i + 1).wait()

                cp_kv(v_hbm, vb, sem_v, i).wait()
                for c in range(5):
                    cp_o(i, c).wait()
                flip(i)

            def compute(n):
                off = n >> 8

                def to_mxu(slot, val):
                    z_s[1 - off, pl.ds(8 * slot, 8), :] = val

                def to_vpu(slot, val):
                    vb[H * RT - off, pl.ds(8 * slot, 8), :] = pltpu.bitcast(val, u32)

                pace = _Pace(to_mxu, to_vpu, z_s)
                prs, os, scored = {}, {}, {0}

                def vpu_part(u):
                    assert u in scored
                    o = None if sm_first else stage_d1()
                    prs[u] = [p_s[...], softmax(s_s[...], 1, pace, k_sm1)]
                    os[u] = o = o or stage_d1()
                    for t in range(3):
                        pace.before_vpu(("o", t), o[0][t], k_fold + dk_fold * t)
                    yield from stage_c(n * unroll + u, prs[u], pace)

                def mxu_part(u):
                    i = n * unroll + u

                    def fin(y):
                        y_s[...] += y if u else jnp.where(i > 0, y, 0.0)

                    q = []
                    pn = jnp.minimum(i + 1, NP - 1)
                    for k in order:
                        if k in "01":
                            yield from stage_b(pn, int(k), pace, lambda: u in prs)
                        elif k == "a":
                            yield from stage_a(jnp.minimum(i + 2, NP - 1), pace, q)
                        elif k == "d":
                            yield from stage_d2(jnp.maximum(i - 1, 0), os[u], pace, fin)
                        elif k == "e":
                            yield from stage_e(i, prs[u], pace)
                        else:
                            spread(q[0], "xy".index(k), pace)
                    scored.add(u + 1)

                mxu = _chain(*[mxu_part(u) for u in range(unroll)])
                vpu = _chain(*[vpu_part(u) for u in range(unroll)])
                nm, nc = (32 + mt) * unroll, 2 * RT * nv * unroll
                done = e = 0
                while done < nc:
                    next(mxu, None)
                    e += 1
                    while done < min(nc, int(e * nc / (nm + lag))):
                        next(vpu, None)
                        done += 1
                    pace.tick(e < nm)
                _run(mxu, vpu)

            def step(n, carry):
                if dma:
                    @pl.loop(ps * unroll, unroll)
                    def _(u):
                        load(n * unroll + u)
                compute(n)
                return carry

            lax.fori_loop(0, nit // unroll, step, 0)

            def fin(y):
                y_s[...] += y
            _run(stage_d2(NP - 1, stage_d1(), free, fin))
            x = x + jnp.sum(y_s[...], axis=0, keepdims=True)
            d, r = _ln(x)

            if dma:
                @pl.when(ps == 0)
                def _():
                    for j in range(2):
                        cp_m(j).wait()
            g = _dot(d, wg[...]) * _wide(r, F // 128)
            u = _dot(d, wu[...]) * _wide(r, F // 128)
            h = (1.0 / (1.0 + jnp.exp(-g))) * u
            if dma:
                @pl.when(ps == 0)
                def _():
                    cp_m(2).wait()
            x = x + _dot(h[:, :F - fl], wd[pl.ds(0, F - fl), :])
            if dma:
                @pl.when(ps == 0)
                def _():
                    cp_m(3).wait()
            x = x + _dot(h[:, F - fl:], wd[pl.ds(F - fl, fl), :])
            return x

        if dma:
            for t in range(3 * NP):
                cp_q(t).wait()
            cp_kv(k_hbm, kb, sem_k, 0).wait()
        x = lax.fori_loop(0, npass, layer, x0)
        o_ref[...] = x[:1].astype(o_ref.dtype)

    @jax.jit
    def fn(A_x, A_k_cache, A_v_cache, A_wq, A_wo, B_x, B_w_gate, B_w_up, B_w_down):
        del B_x
        kt = _raw(jnp.swapaxes(A_k_cache, 2, 3).reshape(H * DH, SK))
        vt = _raw(jnp.swapaxes(A_v_cache, 2, 3).reshape(H * DH, SK))
        hbm = pl.BlockSpec(memory_space=pltpu.HBM)
        out = pl.pallas_call(
            kernel,
            out_shape=jax.ShapeDtypeStruct((1, D), bf16),
            in_specs=[hbm] * 8,
            out_specs=pl.BlockSpec(memory_space=pltpu.VMEM),
            scratch_shapes=[
                pltpu.VMEM((H * RT, W // 32, 128), u32),
                pltpu.VMEM((H * RT + 1, W // 32, 128), u32),
                pltpu.VMEM((3 * NP, D // 2, 128), u32),
                pltpu.VMEM((5 * NP, DH, 128), u32),
                pltpu.VMEM((D, F), bf16),
                pltpu.VMEM((D, F), bf16),
                pltpu.VMEM((F, D), bf16),
                pltpu.VMEM((24, 8, 128), f32),
                pltpu.VMEM((8, 512), f32),
                pltpu.VMEM((8, 512), f32),
                pltpu.VMEM((2 * NT, 8, 128), f32),
                pltpu.VMEM((2 * RT, 8, 128), f32),
                pltpu.VMEM((2, NZ * 8, 128), f32),
                pltpu.VMEM((8, 512), f32),
                pltpu.VMEM((8, D + 384), f32),
                pltpu.VMEM((8, D), f32),
                pltpu.VMEM((1, 2 * D), bf16),
                pltpu.SemaphoreType.DMA((1,)),
                pltpu.SemaphoreType.DMA((1,)),
                pltpu.SemaphoreType.DMA((NP,)),
                pltpu.SemaphoreType.DMA((NP,)),
                pltpu.SemaphoreType.DMA((NP,)),
                pltpu.SemaphoreType.DMA((4,)),
            ],
            compiler_params=pltpu.CompilerParams(
                vmem_limit_bytes=127 * 1024 * 1024, disable_semaphore_checks=True, flags=flags),
        )(A_x.reshape(1, D), kt, vt, A_wq, A_wo, B_w_gate, B_w_up, B_w_down)
        return out.reshape(1, 1, D)

    return fn


_fn = make(**dict({'mt': 4, 'k_m': 5, 'k_acc': 2, 'lag': 4, 'chunk': 3, 'k_q': 16, 'k_sm': 20, 'k_sm1': 18, 'k_fold': 14, 'dk_fold': 3, 'jg': 2, 'sm_first': False, 'k_self': 2, 'order': 'a0x1yed'},look=3,unroll=2))


@jax.jit
def pallas_interleave_layers__sliding_block_cached__glu_gated_glu__decode_kernel(
    A_x, A_k_cache, A_v_cache, A_wq, A_wo, B_x, B_w_gate, B_w_up, B_w_down
):
    return _fn(A_x, A_k_cache, A_v_cache, A_wq, A_wo, B_x, B_w_gate, B_w_up, B_w_down)
```

```python
import jax
import jax.numpy as jnp
from jax import lax
import jax.experimental.pallas as pl
import jax.experimental.pallas.tpu as pltpu

H, DH, SK, D, F = 32, 192, 32768, 640, 1536
W = min(4096, max(256, SK // 4))
NP = H // 2
RT = DH // 8
NT = W // 128
NZ = 16
EPS = 1e-5
bf16, f32, u32 = jnp.bfloat16, jnp.float32, jnp.uint32


def _raw(a):
    r, c = a.shape
    return a.reshape(r // 8, 8, c // 128, 128).transpose(0, 2, 1, 3).reshape(r // 8, c // 128 * 8, 128)


def _ln(x):
    d = x - jnp.sum(x, axis=-1, keepdims=True) * (1.0 / D)
    v = jnp.sum(d * d, axis=-1, keepdims=True) * (1.0 / D)
    return d, jnp.broadcast_to(lax.rsqrt(v + EPS), (8, 128))


def _wide(x, n):
    return jnp.concatenate([x] * n, axis=1)


def _b(x):
    return pltpu.bitcast(x, bf16)


def _dot(a, b):
    return lax.dot_general(a, b, (((1,), (0,)), ((), ())), preferred_element_type=f32)


def _iota(axis):
    return lax.broadcasted_iota(jnp.int32, (8, 128), axis)


def _run(*gens):
    for g in gens:
        for _ in g:
            pass


def _chain(*gens):
    for g in gens:
        yield from g


def _call(f):
    f()
    return
    yield


class _Pace:
    def __init__(self, to_mxu=None, to_vpu=None, z_ref=None):
        self.put, self.z_ref = (to_mxu, to_vpu), z_ref
        self.now, self.due, self.slot = 0, ({}, {}), [0, 0]

    def before_mxu(self, key, val, delay):
        self.due[0][key, self.now] = (self.now + delay, val)

    def before_vpu(self, key, val, delay):
        self.due[1][key, self.now] = (self.now + delay, val)

    def tick(self, mxu):
        self.now += 1
        for w in (0, 1) if mxu else (1,):
            due = self.due[w]
            for key in [k for k, (t, _) in due.items() if t <= self.now]:
                self.slot[w] = (self.slot[w] + 1) % NZ
                self.put[w](self.slot[w], due.pop(key)[1])

    def zero(self):
        if self.z_ref is None:
            return jnp.zeros((8, 128), f32)
        return self.z_ref[0, pl.ds(0, 8), :]


def make(chunk=4, npass=2, look=2, dma=True, lag=5, order="a0xd1ye", tree=False,
         k_acc=2, k_fold=10, dk_fold=3, k_sm=20, k_sm1=60, k_q=12, k_m=5, nit=NP, mt=2, fl=256,
         jg=1, sm_first=False, k_self=1, unroll=1, flags=None):
    nv = (NT - mt) // 2

    def kernel(x_hbm, k_hbm, v_hbm, wq_hbm, wo_hbm, wg_hbm, wu_hbm, wd_hbm, o_ref,
               kb, vb, wq, wo, wg, wu, wd, q_s, s_s, p_s, pb_s, acc_s, z_s, e_s, xn_s, y_s, xb,
               sem_x, sem_q, sem_k, sem_v, sem_o, sem_m):
        k_hbm, v_hbm, wq_hbm, wo_hbm = (r.bitcast(u32) for r in (k_hbm, v_hbm, wq_hbm, wo_hbm))

        def cp_x():
            return pltpu.make_async_copy(x_hbm, xb.at[:, pl.ds(0, D)], sem_x.at[0])

        def cp_q(t):
            return pltpu.make_async_copy(wq_hbm.at[:, pl.ds(128 * t, 128)], wq.at[t], sem_q.at[0])

        def cp_kv(hbm, buf, sem, p):
            rows = pl.ds(p * (2 * RT), 2 * RT)
            return pltpu.make_async_copy(
                hbm.at[rows, pl.ds((SK - W) // 32, W // 32)], buf.at[rows], sem.at[p])

        def cp_o(p, c):
            r0 = pl.multiple_of(p * DH, 64)
            return pltpu.make_async_copy(
                wo_hbm.at[pl.ds(r0, DH), pl.ds(128 * c, 128)], wo.at[p * 5 + c], sem_o.at[p])

        def cp_m(j):
            if j < 2:
                return pltpu.make_async_copy((wg_hbm, wu_hbm)[j], (wg, wu)[j], sem_m.at[j])
            rows = pl.ds(0, F - fl) if j == 2 else pl.ds(F - fl, fl)
            return pltpu.make_async_copy(wd_hbm.at[rows], wd.at[rows], sem_m.at[j])

        def start_step(s):
            cp_kv(v_hbm, vb, sem_v, s).start()
            for c in range(5):
                cp_o(s, c).start()

        if dma:
            cp_x().start()
            for t in range(3 * NP):
                cp_q(t).start()
            cp_kv(k_hbm, kb, sem_k, 0).start()
            for s in range(look):
                cp_kv(k_hbm, kb, sem_k, s + 1).start()
                start_step(s)
            cp_x().wait()
        z_s[0, pl.ds(0, 8), :] = jnp.zeros((8, 128), f32)
        x0 = jnp.broadcast_to(xb[:, pl.ds(0, D)].astype(f32), (8, D))

        def stage_a(p, pace, out):
            q = None
            for k in range(5):
                w = jnp.concatenate([_b(wq[3 * p + t, pl.ds(64 * k, 64), :]) for t in range(3)], axis=1)
                t = _dot(xn_s[:, pl.ds(128 * k, 128)] + pace.zero(), w)
                q = t if q is None else q + t
                pace.before_vpu(0, q[:, :128], k_m)
                yield
            out.append(q * _wide(xn_s[:, pl.ds(D, 128)], 3))

        def spread(q, a, pace):
            lane = _iota(1)
            for g in range(12 * a, 12 * a + 12):
                qt = q[:, 128 * (g // 8):128 * (g // 8 + 1)]
                e = jnp.take_along_axis(qt, ((lane >> 6) << 3) + (lane & 7) + 16 * (g % 8), axis=1)
                q_s[g] = e
                if g % 4 == 3:
                    pace.before_vpu(("q", g), e, k_q)

        def stage_b(p, a, pace, seen=None):
            diag = ((_iota(1) >> 3) & 7) == _iota(0)
            s = None
            for kt in range(12):
                lhs = jnp.where(diag, q_s[12 * a + kt], pace.zero())
                r0 = p * (2 * RT) + a * RT + 2 * kt
                rhs = jnp.concatenate(
                    [_b(kb[pl.ds(r0, 2), pl.ds(32 * c, 32), :].reshape(64, 128)) for c in range(4)],
                    axis=1)
                t = _dot(lhs, rhs)
                s = t if s is None else s + t
                pace.before_vpu(0, s[:, :128], k_m)
                yield
            assert seen is None or seen()
            if a == 1:
                s_s[...] = s
            else:
                p_s[...] = softmax(s, a, pace, k_sm)

        def softmax(s, a, pace, k):
            m = jnp.max(jnp.max(s, axis=1, keepdims=True), axis=0, keepdims=True)
            e = jnp.exp(s - m)
            pace.before_vpu(("sm", a), e[:, :128], k)
            return e

        def row(pr, t):
            return jnp.broadcast_to(pr[t % 8:t % 8 + 1, 128 * (t // 8):128 * (t // 8 + 1)], (8, 128))

        def stage_c(p, prs, pace):
            for a in range(2):
                e = [prs[a][:, 128 * c:128 * (c + 1)] for c in range(4)]
                e_s[:, pl.ds(384 + 128 * a, 128)] = (e[0] + e[1]) + (e[2] + e[3])
                for r in range(0, RT, chunk):
                    r0 = p * (2 * RT) + a * RT + r
                    acc = [None] * chunk
                    for j0 in range(0, nv, jg):
                        js = range(j0, min(j0 + jg, nv))
                        pp = {}
                        for t in range(2 * js[0], 2 * js[-1] + 2):
                            if r == 0:
                                pb_s[NT * a + t] = row(prs[a], t)
                            pp[t] = pb_s[NT * a + t]
                        for n in range(chunk):
                            for j in js:
                                p0, p1 = pp[2 * j], pp[2 * j + 1]
                                v = _b(vb[r0 + n, pl.ds(8 * j, 8), :]).astype(f32)
                                if acc[n] is None:
                                    acc[n] = v[:8] * p0 + v[8:] * p1
                                elif tree:
                                    acc[n] = acc[n] + (v[:8] * p0 + v[8:] * p1)
                                else:
                                    acc[n] = (acc[n] + v[:8] * p0) + v[8:] * p1
                                pace.before_mxu((a, r, n), acc[n], k_acc)
                                if k_self and pace.now + k_self < k_m:
                                    pace.before_vpu("self", acc[n], k_self)
                                yield
                    for n in range(chunk):
                        acc_s[a * RT + r + n] = acc[n]

        def flip(p):
            for u in range(3):
                for j in range(nv, NT // 2):
                    r0 = p * (2 * RT) + 16 * u
                    v = _b(vb[pl.ds(r0, 16), pl.ds(8 * j, 8), :]).astype(f32)
                    for h in range(2):
                        t = v[:, 8 * h:8 * h + 8, :].reshape(128, 128).T.astype(bf16)
                        vb[pl.ds(r0 + 8 * h, 8), pl.ds(8 * j, 8), :] = pltpu.bitcast(t, u32).reshape(8, 8, 128)

        def stage_e(p, prs, pace):
            o = None
            for t in range(NT - mt, NT):
                lhs = jnp.where(_iota(0) < 4, row(prs[0], t), row(prs[1], t)) + pace.zero()
                w = jnp.concatenate(
                    [_b(vb[pl.ds(p * (2 * RT) + 16 * u + 8 * (t % 2), 8), pl.ds(8 * (t // 2), 8), :]
                        .reshape(64, 128)) for u in range(3)], axis=1)
                z = _dot(lhs, w)
                o = z if o is None else o + z
                pace.before_vpu(0, o[:, :128], k_m)
                yield
            if mt:
                e_s[:, pl.ds(0, 384)] = o

        def stage_d1():
            def merge(lo, n):
                if n == 1:
                    return jnp.broadcast_to(jnp.sum(acc_s[lo], axis=1, keepdims=True), (8, 128))
                n //= 2
                return jnp.where((_iota(1) & (8 * n)) == 0, merge(lo, n), merge(lo + n, n))

            tiles = [merge(16 * t, 16) for t in range(3)]
            inv = []
            for a in range(2):
                l = jnp.sum(e_s[:, pl.ds(384 + 128 * a, 128)], axis=0, keepdims=True)
                inv.append(jnp.broadcast_to(1.0 / jnp.sum(l, axis=1, keepdims=True), (8, 128)))
            inv = [inv[0], jnp.where(_iota(1) < 64, inv[0], inv[1]), inv[1]]
            return tiles, (e_s[:, pl.ds(0, 384)] if mt else None), inv

        def stage_d2(p, o, pace, put):
            tiles, extra, inv = o
            y = None
            lane, sub = _iota(1), _iota(0)
            for t in range(3):
                w = jnp.concatenate([_b(wo[5 * p + c, pl.ds(64 * t, 64), :]) for c in range(5)], axis=1)
                lhs = jnp.where((lane & 7) == sub, tiles[t], pace.zero())
                if mt:
                    pick = sub == (0, (lane >> 6) << 2, 4)[t]
                    lhs = lhs + jnp.where(pick, extra[:, 128 * t:128 * (t + 1)], 0.0)
                z = _dot(lhs * inv[t], w)
                y = z if y is None else y + z
                pace.before_vpu(0, y[:, :128], k_m)
                yield
            put(y)

        def layer(ps, x):
            d, r = _ln(x)
            xn_s[:, pl.ds(0, D)] = d
            xn_s[:, pl.ds(D, 128)] = r * (DH ** -0.5)

            free = _Pace()
            q = []
            _run(stage_a(0, free, q))
            spread(q[0], 0, free)
            spread(q[0], 1, free)
            _run(stage_a(1, free, q), stage_b(0, 0, free), stage_b(0, 1, free))
            spread(q[1], 0, free)
            spread(q[1], 1, free)
            acc_s[...] = jnp.zeros(acc_s.shape, f32)
            e_s[...] = jnp.ones(e_s.shape, f32)
            y_s[...] = jnp.zeros(y_s.shape, f32)

            def load(i):
                @pl.when(i + look + 1 < NP)
                def _():
                    cp_kv(k_hbm, kb, sem_k, i + look + 1).start()

                @pl.when(i + look < NP)
                def _():
                    start_step(i + look)

                @pl.when(i + look == NP)
                def _():
                    for j in range(4):
                        cp_m(j).start()

                @pl.when(i + 1 < NP)
                def _():
                    cp_kv(k_hbm, kb, sem_k, i + 1).wait()

                cp_kv(v_hbm, vb, sem_v, i).wait()
                for c in range(5):
                    cp_o(i, c).wait()
                flip(i)

            def compute(n):
                off = n >> 8

                def to_mxu(slot, val):
                    z_s[1 - off, pl.ds(8 * slot, 8), :] = val

                def to_vpu(slot, val):
                    vb[H * RT - off, pl.ds(8 * slot, 8), :] = pltpu.bitcast(val, u32)

                pace = _Pace(to_mxu, to_vpu, z_s)
                prs, os, scored = {}, {}, {0}

                def vpu_part(u):
                    assert u in scored
                    o = None if sm_first else stage_d1()
                    prs[u] = [p_s[...], softmax(s_s[...], 1, pace, k_sm1)]
                    os[u] = o = o or stage_d1()
                    for t in range(3):
                        pace.before_vpu(("o", t), o[0][t], k_fold + dk_fold * t)
                    yield from stage_c(n * unroll + u, prs[u], pace)

                def mxu_part(u):
                    i = n * unroll + u

                    def fin(y):
                        y_s[...] += y if u else jnp.where(i > 0, y, 0.0)

                    q = []
                    pn = jnp.minimum(i + 1, NP - 1)
                    for k in order:
                        if k in "01":
                            yield from stage_b(pn, int(k), pace, lambda: u in prs)
                        elif k == "a":
                            yield from stage_a(jnp.minimum(i + 2, NP - 1), pace, q)
                        elif k == "d":
                            yield from stage_d2(jnp.maximum(i - 1, 0), os[u], pace, fin)
                        elif k == "e":
                            yield from stage_e(i, prs[u], pace)
                        else:
                            spread(q[0], "xy".index(k), pace)
                    scored.add(u + 1)

                mxu = _chain(*[mxu_part(u) for u in range(unroll)])
                vpu = _chain(*[vpu_part(u) for u in range(unroll)])
                nm, nc = (32 + mt) * unroll, 2 * RT * nv * unroll
                done = e = 0
                while done < nc:
                    next(mxu, None)
                    e += 1
                    while done < min(nc, int(e * nc / (nm + lag))):
                        next(vpu, None)
                        done += 1
                    pace.tick(e < nm)
                _run(mxu, vpu)

            def step(n, carry):
                if dma:
                    @pl.loop(ps * unroll, unroll)
                    def _(u):
                        load(n * unroll + u)
                compute(n)
                return carry

            lax.fori_loop(0, nit // unroll, step, 0)

            def fin(y):
                y_s[...] += y
            _run(stage_d2(NP - 1, stage_d1(), free, fin))
            x = x + jnp.sum(y_s[...], axis=0, keepdims=True)
            d, r = _ln(x)

            if dma:
                @pl.when(ps == 0)
                def _():
                    for j in range(2):
                        cp_m(j).wait()
            g = _dot(d, wg[...]) * _wide(r, F // 128)
            u = _dot(d, wu[...]) * _wide(r, F // 128)
            h = (1.0 / (1.0 + jnp.exp(-g))) * u
            if dma:
                @pl.when(ps == 0)
                def _():
                    cp_m(2).wait()
            x = x + _dot(h[:, :F - fl], wd[pl.ds(0, F - fl), :])
            if dma:
                @pl.when(ps == 0)
                def _():
                    cp_m(3).wait()
            x = x + _dot(h[:, F - fl:], wd[pl.ds(F - fl, fl), :])
            return x

        if dma:
            for t in range(3 * NP):
                cp_q(t).wait()
            cp_kv(k_hbm, kb, sem_k, 0).wait()
        x = lax.fori_loop(0, npass, layer, x0)
        o_ref[...] = x[:1].astype(o_ref.dtype)

    @jax.jit
    def fn(A_x, A_k_cache, A_v_cache, A_wq, A_wo, B_x, B_w_gate, B_w_up, B_w_down):
        del B_x
        kt = _raw(jnp.swapaxes(A_k_cache, 2, 3).reshape(H * DH, SK))
        vt = _raw(jnp.swapaxes(A_v_cache, 2, 3).reshape(H * DH, SK))
        hbm = pl.BlockSpec(memory_space=pltpu.HBM)
        out = pl.pallas_call(
            kernel,
            out_shape=jax.ShapeDtypeStruct((1, D), bf16),
            in_specs=[hbm] * 8,
            out_specs=pl.BlockSpec(memory_space=pltpu.VMEM),
            scratch_shapes=[
                pltpu.VMEM((H * RT, W // 32, 128), u32),
                pltpu.VMEM((H * RT + 1, W // 32, 128), u32),
                pltpu.VMEM((3 * NP, D // 2, 128), u32),
                pltpu.VMEM((5 * NP, DH, 128), u32),
                pltpu.VMEM((D, F), bf16),
                pltpu.VMEM((D, F), bf16),
                pltpu.VMEM((F, D), bf16),
                pltpu.VMEM((24, 8, 128), f32),
                pltpu.VMEM((8, 512), f32),
                pltpu.VMEM((8, 512), f32),
                pltpu.VMEM((2 * NT, 8, 128), f32),
                pltpu.VMEM((2 * RT, 8, 128), f32),
                pltpu.VMEM((2, NZ * 8, 128), f32),
                pltpu.VMEM((8, 1024), f32),
                pltpu.VMEM((8, D + 384), f32),
                pltpu.VMEM((8, D), f32),
                pltpu.VMEM((1, 2 * D), bf16),
                pltpu.SemaphoreType.DMA((1,)),
                pltpu.SemaphoreType.DMA((1,)),
                pltpu.SemaphoreType.DMA((NP,)),
                pltpu.SemaphoreType.DMA((NP,)),
                pltpu.SemaphoreType.DMA((NP,)),
                pltpu.SemaphoreType.DMA((4,)),
            ],
            compiler_params=pltpu.CompilerParams(
                vmem_limit_bytes=127 * 1024 * 1024, disable_semaphore_checks=True, flags=flags),
        )(A_x.reshape(1, D), kt, vt, A_wq, A_wo, B_w_gate, B_w_up, B_w_down)
        return out.reshape(1, 1, D)

    return fn


_fn = make(**{'chunk': 2, 'dk_fold': 2, 'jg': 2, 'k_acc': 2, 'k_fold': 14, 'k_m': 6, 'k_q': 16, 'k_self': 5, 'k_sm': 16, 'k_sm1': 10, 'lag': 5, 'look': 3, 'mt': 4, 'order': '0ax1yed', 'sm_first': False, 'unroll': 2})


@jax.jit
def pallas_interleave_layers__sliding_block_cached__glu_gated_glu__decode_kernel(
    A_x, A_k_cache, A_v_cache, A_wq, A_wo, B_x, B_w_gate, B_w_up, B_w_down
):
    return _fn(A_x, A_k_cache, A_v_cache, A_wq, A_wo, B_x, B_w_gate, B_w_up, B_w_down)
```

```python
import jax
import jax.numpy as jnp
from jax import lax
import jax.experimental.pallas as pl
import jax.experimental.pallas.tpu as pltpu

H, DH, SK, D, F = 32, 192, 32768, 640, 1536
W = min(4096, max(256, SK // 4))
EPS = 1e-5
NP = H // 2
RT = DH // 8
NT = W // 128
MT = 4
NV = (NT - MT) // 2
LAYERS = 2
UNROLL = 2
LOOK = 2
FL = 256
NZ = 16
bf16, f32, u32 = jnp.bfloat16, jnp.float32, jnp.uint32


def _tiles(a):
    r, c = a.shape
    a = a.reshape(r // 8, 8, c // 128, 128).transpose(0, 2, 1, 3)
    return a.reshape(r // 8, c // 128 * 8, 128)


def _layernorm(x):
    d = x - jnp.sum(x, axis=-1, keepdims=True) * (1.0 / D)
    v = jnp.sum(d * d, axis=-1, keepdims=True) * (1.0 / D)
    return d, jnp.broadcast_to(lax.rsqrt(v + EPS), (8, 128))


def _wide(x, n):
    return jnp.concatenate([x] * n, axis=1)


def _b(x):
    return pltpu.bitcast(x, bf16)


def _dot(a, b):
    return lax.dot_general(a, b, (((1,), (0,)), ((), ())), preferred_element_type=f32)


def _iota(axis):
    return lax.broadcasted_iota(jnp.int32, (8, 128), axis)


def _run(*gens):
    for g in gens:
        for _ in g:
            pass


def _chain(*gens):
    for g in gens:
        yield from g


class _Pace:
    def __init__(self, to_mxu=None, to_vpu=None, z_ref=None):
        self.put, self.z_ref = (to_mxu, to_vpu), z_ref
        self.now, self.due, self.slot = 0, ({}, {}), [0, 0]

    def before_mxu(self, key, val, delay):
        self.due[0][key, self.now] = (self.now + delay, val)

    def before_vpu(self, key, val, delay):
        self.due[1][key, self.now] = (self.now + delay, val)

    def tick(self, mxu):
        self.now += 1
        for w in (0, 1) if mxu else (1,):
            due = self.due[w]
            for key in [k for k, (t, _) in due.items() if t <= self.now]:
                self.slot[w] = (self.slot[w] + 1) % NZ
                self.put[w](self.slot[w], due.pop(key)[1])

    def zero(self):
        if self.z_ref is None:
            return jnp.zeros((8, 128), f32)
        return self.z_ref[0, pl.ds(0, 8), :]


K_MXU, K_ACC, K_SELF, K_Q, K_SM0, K_SM1, K_FOLD, LAG = 6, 2, 5, 16, 16, 10, 14, 5
M_STEPS = 5 + 24 + 3 + MT
V_STEPS = 2 * RT * NV


def _kernel(x_hbm, k_hbm, v_hbm, wq_hbm, wo_hbm, wg_hbm, wu_hbm, wd_hbm, o_ref,
            kb, vb, wq, wo, wg, wu, wd, q_s, s_s, p_s, pb_s, acc_s, z_s, e_s, xn_s, y_s, xb,
            sem_x, sem_q, sem_k, sem_v, sem_o, sem_m):
    k_hbm, v_hbm, wq_hbm, wo_hbm = (r.bitcast(u32) for r in (k_hbm, v_hbm, wq_hbm, wo_hbm))

    def cp_x():
        return pltpu.make_async_copy(x_hbm, xb.at[:, pl.ds(0, D)], sem_x.at[0])

    def cp_q(t):
        return pltpu.make_async_copy(wq_hbm.at[:, pl.ds(128 * t, 128)], wq.at[t], sem_q.at[0])

    def cp_kv(hbm, buf, sem, p):
        rows = pl.ds(p * (2 * RT), 2 * RT)
        return pltpu.make_async_copy(
            hbm.at[rows, pl.ds((SK - W) // 32, W // 32)], buf.at[rows], sem.at[p])

    def cp_o(p, c):
        r0 = pl.multiple_of(p * DH, 64)
        return pltpu.make_async_copy(
            wo_hbm.at[pl.ds(r0, DH), pl.ds(128 * c, 128)], wo.at[p * 5 + c], sem_o.at[p])

    def cp_m(j):
        if j < 2:
            return pltpu.make_async_copy((wg_hbm, wu_hbm)[j], (wg, wu)[j], sem_m.at[j])
        rows = pl.ds(0, F - FL) if j == 2 else pl.ds(F - FL, FL)
        return pltpu.make_async_copy(wd_hbm.at[rows], wd.at[rows], sem_m.at[j])

    def start_vo(p):
        cp_kv(v_hbm, vb, sem_v, p).start()
        for c in range(5):
            cp_o(p, c).start()

    cp_x().start()
    for t in range(3 * NP):
        cp_q(t).start()
    cp_kv(k_hbm, kb, sem_k, 0).start()
    for p in range(LOOK):
        cp_kv(k_hbm, kb, sem_k, p + 1).start()
        start_vo(p)
    cp_x().wait()
    z_s[0, pl.ds(0, 8), :] = jnp.zeros((8, 128), f32)
    x0 = jnp.broadcast_to(xb[:, pl.ds(0, D)].astype(f32), (8, D))

    def project(p, pace, out):
        q = None
        for k in range(5):
            w = jnp.concatenate([_b(wq[3 * p + t, pl.ds(64 * k, 64), :]) for t in range(3)], axis=1)
            t = _dot(xn_s[:, pl.ds(128 * k, 128)] + pace.zero(), w)
            q = t if q is None else q + t
            pace.before_vpu(0, q[:, :128], K_MXU)
            yield
        out.append(q * _wide(xn_s[:, pl.ds(D, 128)], 3))

    def spread(q, a, pace):
        lane = _iota(1)
        for g in range(12 * a, 12 * a + 12):
            qt = q[:, 128 * (g // 8):128 * (g // 8 + 1)]
            e = jnp.take_along_axis(qt, ((lane >> 6) << 3) + (lane & 7) + 16 * (g % 8), axis=1)
            q_s[g] = e
            if g % 4 == 3:
                pace.before_vpu(("q", g), e, K_Q)

    def scores(p, a, pace, consumed=lambda: True):
        diag = ((_iota(1) >> 3) & 7) == _iota(0)
        s = None
        for kt in range(12):
            lhs = jnp.where(diag, q_s[12 * a + kt], pace.zero())
            r0 = p * (2 * RT) + a * RT + 2 * kt
            rhs = jnp.concatenate(
                [_b(kb[pl.ds(r0, 2), pl.ds(32 * c, 32), :].reshape(64, 128)) for c in range(4)],
                axis=1)
            t = _dot(lhs, rhs)
            s = t if s is None else s + t
            pace.before_vpu(0, s[:, :128], K_MXU)
            yield
        assert consumed()
        if a == 1:
            s_s[...] = s
        else:
            p_s[...] = softmax_numerator(s, a, pace, K_SM0)

    def softmax_numerator(s, a, pace, delay):
        m = jnp.max(jnp.max(s, axis=1, keepdims=True), axis=0, keepdims=True)
        e = jnp.exp(s - m)
        pace.before_vpu(("sm", a), e[:, :128], delay)
        return e

    def row(pr, t):
        return jnp.broadcast_to(pr[t % 8:t % 8 + 1, 128 * (t // 8):128 * (t // 8 + 1)], (8, 128))

    def pv_vpu(p, prs, pace):
        for a in range(2):
            e = [prs[a][:, 128 * c:128 * (c + 1)] for c in range(4)]
            e_s[:, pl.ds(384 + 128 * a, 128)] = (e[0] + e[1]) + (e[2] + e[3])
            for r in range(0, RT, 2):
                r0 = p * (2 * RT) + a * RT + r
                acc = [None, None]
                for j0 in range(0, NV, 2):
                    pp = {}
                    for t in range(2 * j0, 2 * j0 + 4):
                        if r == 0:
                            pb_s[NT * a + t] = row(prs[a], t)
                        pp[t] = pb_s[NT * a + t]
                    for n in range(2):
                        for j in (j0, j0 + 1):
                            v = _b(vb[r0 + n, pl.ds(8 * j, 8), :]).astype(f32)
                            if acc[n] is None:
                                acc[n] = v[:8] * pp[2 * j] + v[8:] * pp[2 * j + 1]
                            else:
                                acc[n] = (acc[n] + v[:8] * pp[2 * j]) + v[8:] * pp[2 * j + 1]
                            pace.before_mxu((a, r, n), acc[n], K_ACC)
                            if pace.now + K_SELF < K_MXU:
                                pace.before_vpu("self", acc[n], K_SELF)
                            yield
                for n in range(2):
                    acc_s[a * RT + r + n] = acc[n]

    def flip(p):
        for u in range(3):
            for j in range(NV, NT // 2):
                r0 = p * (2 * RT) + 16 * u
                v = _b(vb[pl.ds(r0, 16), pl.ds(8 * j, 8), :]).astype(f32)
                for h in range(2):
                    t = v[:, 8 * h:8 * h + 8, :].reshape(128, 128).T.astype(bf16)
                    vb[pl.ds(r0 + 8 * h, 8), pl.ds(8 * j, 8), :] = (
                        pltpu.bitcast(t, u32).reshape(8, 8, 128))

    def pv_mxu(p, prs, pace):
        o = None
        for t in range(NT - MT, NT):
            lhs = jnp.where(_iota(0) < 4, row(prs[0], t), row(prs[1], t)) + pace.zero()
            r0 = p * (2 * RT) + 8 * (t % 2)
            w = jnp.concatenate(
                [_b(vb[pl.ds(r0 + 16 * u, 8), pl.ds(8 * (t // 2), 8), :].reshape(64, 128))
                 for u in range(3)], axis=1)
            z = _dot(lhs, w)
            o = z if o is None else o + z
            pace.before_vpu(0, o[:, :128], K_MXU)
            yield
        e_s[:, pl.ds(0, 384)] = o

    def fold():
        def merge(lo, n):
            if n == 1:
                return jnp.broadcast_to(jnp.sum(acc_s[lo], axis=1, keepdims=True), (8, 128))
            n //= 2
            return jnp.where((_iota(1) & (8 * n)) == 0, merge(lo, n), merge(lo + n, n))

        tiles = [merge(16 * t, 16) for t in range(3)]
        inv = []
        for a in range(2):
            l = jnp.sum(e_s[:, pl.ds(384 + 128 * a, 128)], axis=0, keepdims=True)
            inv.append(jnp.broadcast_to(1.0 / jnp.sum(l, axis=1, keepdims=True), (8, 128)))
        inv = [inv[0], jnp.where(_iota(1) < 64, inv[0], inv[1]), inv[1]]
        return tiles, e_s[:, pl.ds(0, 384)], inv

    def out_project(p, o, pace, put):
        tiles, extra, inv = o
        y = None
        lane, sub = _iota(1), _iota(0)
        for t in range(3):
            w = jnp.concatenate([_b(wo[5 * p + c, pl.ds(64 * t, 64), :]) for c in range(5)], axis=1)
            lhs = jnp.where((lane & 7) == sub, tiles[t], pace.zero())
            pick = sub == (0, (lane >> 6) << 2, 4)[t]
            lhs = lhs + jnp.where(pick, extra[:, 128 * t:128 * (t + 1)], 0.0)
            z = _dot(lhs * inv[t], w)
            y = z if y is None else y + z
            pace.before_vpu(0, y[:, :128], K_MXU)
            yield
        put(y)

    def load(i):
        @pl.when(i + LOOK + 1 < NP)
        def _():
            cp_kv(k_hbm, kb, sem_k, i + LOOK + 1).start()

        @pl.when(i + LOOK < NP)
        def _():
            start_vo(i + LOOK)

        @pl.when(i + LOOK == NP)
        def _():
            for j in range(4):
                cp_m(j).start()

        @pl.when(i + 1 < NP)
        def _():
            cp_kv(k_hbm, kb, sem_k, i + 1).wait()

        cp_kv(v_hbm, vb, sem_v, i).wait()
        for c in range(5):
            cp_o(i, c).wait()
        flip(i)

    def compute(n):
        off = n >> 8

        def to_mxu(slot, val):
            z_s[1 - off, pl.ds(8 * slot, 8), :] = val

        def to_vpu(slot, val):
            vb[H * RT - off, pl.ds(8 * slot, 8), :] = pltpu.bitcast(val, u32)

        pace = _Pace(to_mxu, to_vpu, z_s)
        prs, outs, scored = {}, {}, [0]

        def vpu_part(u):
            assert u in scored
            outs[u] = fold()
            prs[u] = [p_s[...], softmax_numerator(s_s[...], 1, pace, K_SM1)]
            for t in range(3):
                pace.before_vpu(("o", t), outs[u][0][t], K_FOLD + 2 * t)
            yield from pv_vpu(n * UNROLL + u, prs[u], pace)

        def mxu_part(u):
            i = n * UNROLL + u

            def add(y):
                y_s[...] += y if u else jnp.where(i > 0, y, 0.0)

            q = []
            nxt = jnp.minimum(i + 1, NP - 1)
            yield from scores(nxt, 0, pace, lambda: u in prs)
            yield from project(jnp.minimum(i + 2, NP - 1), pace, q)
            spread(q[0], 0, pace)
            yield from scores(nxt, 1, pace, lambda: u in prs)
            spread(q[0], 1, pace)
            yield from pv_mxu(i, prs[u], pace)
            yield from out_project(jnp.maximum(i - 1, 0), outs[u], pace, add)
            scored.append(u + 1)

        mxu = _chain(*[mxu_part(u) for u in range(UNROLL)])
        vpu = _chain(*[vpu_part(u) for u in range(UNROLL)])
        nm, nv = M_STEPS * UNROLL, V_STEPS * UNROLL
        done = e = 0
        while done < nv:
            next(mxu, None)
            e += 1
            while done < min(nv, e * nv // (nm + LAG)):
                next(vpu, None)
                done += 1
            pace.tick(e < nm)
        _run(mxu, vpu)

    def finish(x, wait):
        y = []
        _run(out_project(NP - 1, fold(), _Pace(), y.append))
        x = x + jnp.sum(y_s[...] + y[0], axis=0, keepdims=True)
        d, r = _layernorm(x)
        h = []
        if wait:
            cp_m(0).wait()
            cp_m(1).wait()
        for c in range(0, F, 256):
            w = jnp.concatenate([wg[:, pl.ds(c, 256)], wu[:, pl.ds(c, 256)]], axis=1)
            gu = _dot(d, w) * _wide(r, 4)
            h.append((1.0 / (1.0 + jnp.exp(-gu[:, :256]))) * gu[:, 256:])
        h = jnp.concatenate(h, axis=1)
        if wait:
            cp_m(2).wait()
        x = x + _dot(h[:, :F - FL], wd[pl.ds(0, F - FL), :])
        if wait:
            cp_m(3).wait()
        return x + _dot(h[:, F - FL:], wd[pl.ds(F - FL, FL), :])

    def layer(li, x):
        d, r = _layernorm(x)
        xn_s[:, pl.ds(0, D)] = d
        xn_s[:, pl.ds(D, 128)] = r * (DH ** -0.5)

        free = _Pace()
        q = []
        _run(project(0, free, q))
        spread(q[0], 0, free)
        spread(q[0], 1, free)
        _run(project(1, free, q), scores(0, 0, free), scores(0, 1, free))
        spread(q[1], 0, free)
        spread(q[1], 1, free)
        acc_s[...] = jnp.zeros(acc_s.shape, f32)
        e_s[...] = jnp.ones(e_s.shape, f32)
        y_s[...] = jnp.zeros(y_s.shape, f32)

        def step(n, carry):
            @pl.loop(li * UNROLL, UNROLL)
            def _(u):
                load(n * UNROLL + u)

            compute(n)
            return carry

        lax.fori_loop(0, NP // UNROLL, step, 0)
        return lax.cond(li == 0, lambda x: finish(x, True), lambda x: finish(x, False), x)

    for t in range(3 * NP):
        cp_q(t).wait()
    cp_kv(k_hbm, kb, sem_k, 0).wait()
    x = lax.fori_loop(0, LAYERS, layer, x0)
    o_ref[...] = x[:1].astype(o_ref.dtype)


@jax.jit
def pallas_interleave_layers__sliding_block_cached__glu_gated_glu__decode_kernel(
    A_x: jax.Array,
    A_k_cache: jax.Array,
    A_v_cache: jax.Array,
    A_wq: jax.Array,
    A_wo: jax.Array,
    B_x: jax.Array,
    B_w_gate: jax.Array,
    B_w_up: jax.Array,
    B_w_down: jax.Array,
):
    del B_x
    assert A_k_cache.shape == A_v_cache.shape == (1, H, SK, DH)
    kt = _tiles(jnp.swapaxes(A_k_cache, 2, 3).reshape(H * DH, SK))
    vt = _tiles(jnp.swapaxes(A_v_cache, 2, 3).reshape(H * DH, SK))
    out = pl.pallas_call(
        _kernel,
        out_shape=jax.ShapeDtypeStruct((1, D), A_x.dtype),
        in_specs=[pl.BlockSpec(memory_space=pltpu.HBM)] * 8,
        out_specs=pl.BlockSpec(memory_space=pltpu.VMEM),
        scratch_shapes=[
            pltpu.VMEM((H * RT, W // 32, 128), u32),
            pltpu.VMEM((H * RT + 1, W // 32, 128), u32),
            pltpu.VMEM((3 * NP, D // 2, 128), u32),
            pltpu.VMEM((5 * NP, DH, 128), u32),
            pltpu.VMEM((D, F), bf16),
            pltpu.VMEM((D, F), bf16),
            pltpu.VMEM((F, D), bf16),
            pltpu.VMEM((24, 8, 128), f32),
            pltpu.VMEM((8, 512), f32),
            pltpu.VMEM((8, 512), f32),
            pltpu.VMEM((2 * NT, 8, 128), f32),
            pltpu.VMEM((2 * RT, 8, 128), f32),
            pltpu.VMEM((2, NZ * 8, 128), f32),
            pltpu.VMEM((8, 1024), f32),
            pltpu.VMEM((8, D + 384), f32),
            pltpu.VMEM((8, D), f32),
            pltpu.VMEM((1, 2 * D), bf16),
            pltpu.SemaphoreType.DMA((1,)),
            pltpu.SemaphoreType.DMA((1,)),
            pltpu.SemaphoreType.DMA((NP,)),
            pltpu.SemaphoreType.DMA((NP,)),
            pltpu.SemaphoreType.DMA((NP,)),
            pltpu.SemaphoreType.DMA((4,)),
        ],
        compiler_params=pltpu.CompilerParams(
            vmem_limit_bytes=127 * 1024 * 1024, disable_semaphore_checks=True),
    )(A_x.reshape(1, D), kt, vt, A_wq, A_wo, B_w_gate, B_w_up, B_w_down)
    return out.reshape(1, 1, D)
```

```python
import jax
import jax.numpy as jnp
from jax import lax
import jax.experimental.pallas as pl
import jax.experimental.pallas.tpu as pltpu

H, DH, SK, D, F = 32, 192, 32768, 640, 1536
W = min(4096, max(256, SK // 4))
NP = H // 2
RT = DH // 8
NT = W // 128
NZ = 16
EPS = 1e-5
bf16, f32, u32 = jnp.bfloat16, jnp.float32, jnp.uint32


def _raw(a):
    r, c = a.shape
    return a.reshape(r // 8, 8, c // 128, 128).transpose(0, 2, 1, 3).reshape(r // 8, c // 128 * 8, 128)


def _ln(x):
    d = x - jnp.sum(x, axis=-1, keepdims=True) * (1.0 / D)
    v = jnp.sum(d * d, axis=-1, keepdims=True) * (1.0 / D)
    return d, jnp.broadcast_to(lax.rsqrt(v + EPS), (8, 128))


def _wide(x, n):
    return jnp.concatenate([x] * n, axis=1)


def _b(x):
    return pltpu.bitcast(x, bf16)


def _dot(a, b):
    return lax.dot_general(a, b, (((1,), (0,)), ((), ())), preferred_element_type=f32)


def _iota(axis):
    return lax.broadcasted_iota(jnp.int32, (8, 128), axis)


def _run(*gens):
    for g in gens:
        for _ in g:
            pass


def _chain(*gens):
    for g in gens:
        yield from g


def _call(f):
    f()
    return
    yield


class _Pace:
    def __init__(self, to_mxu=None, to_vpu=None, z_ref=None):
        self.put, self.z_ref = (to_mxu, to_vpu), z_ref
        self.now, self.due, self.slot = 0, ({}, {}), [0, 0]

    def before_mxu(self, key, val, delay):
        self.due[0][key, self.now] = (self.now + delay, val)

    def before_vpu(self, key, val, delay):
        self.due[1][key, self.now] = (self.now + delay, val)

    def tick(self, mxu, vpu):
        self.now += 1
        for w in [w for w, on in enumerate((mxu, vpu)) if on]:
            due = self.due[w]
            for key in [k for k, (t, _) in due.items() if t <= self.now]:
                self.slot[w] = (self.slot[w] + 1) % NZ
                self.put[w](self.slot[w], due.pop(key)[1])

    def zero(self):
        if self.z_ref is None:
            return jnp.zeros((8, 128), f32)
        return self.z_ref[0, pl.ds(0, 8), :]


def make(chunk=4, npass=2, look=2, dma=True, lag=5, order="a0xd1ye", tree=False,
         k_acc=2, k_fold=10, dk_fold=3, k_sm=20, k_sm1=60, k_q=12, k_m=5, nit=NP, mt=2, fl=256,
         jg=1, ucols=(2, 6, 11), vm=127, sk=0, mtb=4, gl=False, ez=1, ev=1, gw=256, sm_first=False, k_self=1, unroll=1, flags=None):
    mts = [mt, mtb] * (unroll // 2)
    ucols = list(ucols)
    nu = len(ucols)

    def kernel(x_hbm, k_hbm, v_hbm, wq_hbm, wo_hbm, wg_hbm, wu_hbm, wd_hbm, o_ref,
               kb, vb, wq, wo, wg, wu, wd, q_s, s_s, p_s, pb_s, acc_s, z_s, e_s, xn_s, y_s, xb,
               sem_x, sem_q, sem_k, sem_v, sem_o, sem_m):
        k_hbm, v_hbm, wq_hbm, wo_hbm = (r.bitcast(u32) for r in (k_hbm, v_hbm, wq_hbm, wo_hbm))

        def cp_x():
            return pltpu.make_async_copy(x_hbm, xb.at[:, pl.ds(0, D)], sem_x.at[0])

        def cp_q(t):
            return pltpu.make_async_copy(wq_hbm.at[:, pl.ds(128 * t, 128)], wq.at[t], sem_q.at[0])

        def cp_kv(hbm, buf, sem, p):
            rows = pl.ds(p * (2 * RT), 2 * RT)
            return pltpu.make_async_copy(
                hbm.at[rows, pl.ds((SK - W) // 32, W // 32)], buf.at[rows], sem.at[p])

        def cp_o(p, c):
            r0 = pl.multiple_of(p * DH, 64)
            return pltpu.make_async_copy(
                wo_hbm.at[pl.ds(r0, DH), pl.ds(128 * c, 128)], wo.at[p * 5 + c], sem_o.at[p])

        def cp_m(j):
            if j < 2:
                return pltpu.make_async_copy((wg_hbm, wu_hbm)[j], (wg, wu)[j], sem_m.at[j])
            rows = pl.ds(0, F - fl) if j == 2 else pl.ds(F - fl, fl)
            return pltpu.make_async_copy(wd_hbm.at[rows], wd.at[rows], sem_m.at[j])

        def start_step(s):
            cp_kv(v_hbm, vb, sem_v, s).start()
            for c in range(5):
                cp_o(s, c).start()

        if dma:
            cp_x().start()
            for t in range(3 * NP):
                cp_q(t).start()
            cp_kv(k_hbm, kb, sem_k, 0).start()
            for s in range(look):
                cp_kv(k_hbm, kb, sem_k, s + 1).start()
                start_step(s)
            cp_x().wait()
        z_s[0, pl.ds(0, 8), :] = jnp.zeros((8, 128), f32)
        x0 = jnp.broadcast_to(xb[:, pl.ds(0, D)].astype(f32), (8, D))

        def stage_a(p, pace, out):
            q = None
            for k in range(5):
                w = jnp.concatenate([_b(wq[3 * p + t, pl.ds(64 * k, 64), :]) for t in range(3)], axis=1)
                t = _dot(xn_s[:, pl.ds(128 * k, 128)] + pace.zero(), w)
                q = t if q is None else q + t
                pace.before_vpu(0, q[:, -128:] if gl else q[:, :128], k_m)
                yield
            out.append(q * _wide(xn_s[:, pl.ds(D, 128)], 3))

        def spread(q, a, pace):
            lane = _iota(1)
            for g in range(12 * a, 12 * a + 12):
                qt = q[:, 128 * (g // 8):128 * (g // 8 + 1)]
                e = jnp.take_along_axis(qt, ((lane >> 6) << 3) + (lane & 7) + 16 * (g % 8), axis=1)
                q_s[g] = e
                if g % 4 == 3:
                    pace.before_vpu(("q", g), e, k_q)

        def stage_b(p, a, pace, seen=None):
            diag = ((_iota(1) >> 3) & 7) == _iota(0)
            s = None
            for kt in range(12):
                lhs = jnp.where(diag, q_s[12 * a + kt], pace.zero())
                r0 = p * (2 * RT) + a * RT + 2 * kt
                rhs = jnp.concatenate(
                    [_b(kb[pl.ds(r0, 2), pl.ds(32 * c, 32), :].reshape(64, 128)) for c in range(4)],
                    axis=1)
                t = _dot(lhs, rhs)
                s = t if s is None else s + t
                pace.before_vpu(0, s[:, -128:] if gl else s[:, :128], k_m)
                yield
            assert seen is None or seen()
            if a == 1:
                s_s[...] = s
            else:
                p_s[...] = softmax(s, a, pace, k_sm)

        def softmax(s, a, pace, k):
            m = jnp.max(jnp.max(s, axis=1, keepdims=True), axis=0, keepdims=True)
            e = jnp.exp(s - m)
            pace.before_vpu(("sm", a), e[:, :128], k)
            return e

        def row(pr, t):
            return jnp.broadcast_to(pr[t % 8:t % 8 + 1, 128 * (t // 8):128 * (t // 8 + 1)], (8, 128))

        def upper(p, rt, ju):
            k = rt * nu + ju
            return H * RT + 1 + p * (3 * nu) + k // 16, pl.ds(8 * (k % 16), 8), slice(None)

        def widen(p):
            for r in range(0, 2 * RT, 8):
                vs = {(rt, ju): _b(vb[p * (2 * RT) + rt, pl.ds(8 * j, 8), :]).astype(f32)
                      for rt in range(r, r + 8) for ju, j in enumerate(ucols)}
                for (rt, ju), v in vs.items():
                    vb[p * (2 * RT) + rt, pl.ds(8 * ucols[ju], 8), :] = pltpu.bitcast(v[:8], u32)
                    vb[upper(p, rt, ju)] = pltpu.bitcast(v[8:], u32)

        def stage_c(p, prs, pace, mt):
            nv = (NT - mt) // 2
            have = set()
            for a in range(2):
                e = [prs[a][:, 128 * c:128 * (c + 1)] for c in range(4)]
                e_s[:, pl.ds(384 + 128 * a, 128)] = (e[0] + e[1]) + (e[2] + e[3])
                for r in range(0, RT, chunk):
                    r0 = p * (2 * RT) + a * RT + r
                    acc = [None] * chunk
                    for j0 in range(0, nv, jg):
                        for n in range(chunk):
                            for j in range(j0, min(j0 + jg, nv)):
                                j = (j + n * sk) % nv
                                for t in (2 * j, 2 * j + 1):
                                    if (a, t) not in have:
                                        have.add((a, t))
                                        pb_s[NT * a + t] = row(prs[a], t)
                                p0, p1 = pb_s[NT * a + 2 * j], pb_s[NT * a + 2 * j + 1]
                                if j in ucols:
                                    lo = pltpu.bitcast(vb[r0 + n, pl.ds(8 * j, 8), :], f32)
                                    hi = pltpu.bitcast(vb[upper(p, a * RT + r + n, ucols.index(j))], f32)
                                else:
                                    v = _b(vb[r0 + n, pl.ds(8 * j, 8), :]).astype(f32)
                                    lo, hi = v[:8], v[8:]
                                if acc[n] is None:
                                    acc[n] = lo * p0 + hi * p1
                                elif tree:
                                    acc[n] = acc[n] + (lo * p0 + hi * p1)
                                else:
                                    acc[n] = (acc[n] + lo * p0) + hi * p1
                                pace.before_mxu((a, r, n), acc[n], k_acc)
                                if k_self and pace.now + k_self < k_m:
                                    pace.before_vpu("self", acc[n], k_self)
                                yield
                    for n in range(chunk):
                        acc_s[a * RT + r + n] = acc[n]

        def flip(p, mt):
            @pl.loop((NT - mt) // 2, NT // 2)
            def _(j):
                cols = pl.ds(pl.multiple_of(8 * j, 8), 8)
                vs = [_b(vb[pl.ds(p * (2 * RT) + 16 * u, 16), cols, :]).astype(f32) for u in range(3)]
                ts = [v[:, 8 * h:8 * h + 8, :].reshape(128, 128).T.astype(bf16) for v in vs for h in range(2)]
                for n, t in enumerate(ts):
                    vb[pl.ds(p * (2 * RT) + 8 * n, 8), cols, :] = pltpu.bitcast(t, u32).reshape(8, 8, 128)

        def stage_e(p, prs, pace, mt):
            o = None
            for t in range(NT - mt, NT):
                lhs = jnp.where(_iota(0) < 4, row(prs[0], t), row(prs[1], t)) + pace.zero()
                w = jnp.concatenate(
                    [_b(vb[pl.ds(p * (2 * RT) + 16 * u + 8 * (t % 2), 8), pl.ds(8 * (t // 2), 8), :]
                        .reshape(64, 128)) for u in range(3)], axis=1)
                z = _dot(lhs, w)
                o = z if o is None else o + z
                pace.before_vpu(0, o[:, -128:] if gl else o[:, :128], k_m)
                yield
            if mt:
                e_s[:, pl.ds(0, 384)] = o

        def stage_d1():
            def merge(lo, n):
                if n == 1:
                    return jnp.broadcast_to(jnp.sum(acc_s[lo], axis=1, keepdims=True), (8, 128))
                n //= 2
                return jnp.where((_iota(1) & (8 * n)) == 0, merge(lo, n), merge(lo + n, n))

            tiles = [merge(16 * t, 16) for t in range(3)]
            inv = []
            for a in range(2):
                l = jnp.sum(e_s[:, pl.ds(384 + 128 * a, 128)], axis=0, keepdims=True)
                inv.append(jnp.broadcast_to(1.0 / jnp.sum(l, axis=1, keepdims=True), (8, 128)))
            inv = [inv[0], jnp.where(_iota(1) < 64, inv[0], inv[1]), inv[1]]
            return tiles, (e_s[:, pl.ds(0, 384)] if mt else None), inv

        def stage_d2(p, o, pace, put):
            tiles, extra, inv = o
            y = None
            lane, sub = _iota(1), _iota(0)
            for t in range(3):
                w = jnp.concatenate([_b(wo[5 * p + c, pl.ds(64 * t, 64), :]) for c in range(5)], axis=1)
                lhs = jnp.where((lane & 7) == sub, tiles[t], pace.zero())
                if mt:
                    pick = sub == (0, (lane >> 6) << 2, 4)[t]
                    lhs = lhs + jnp.where(pick, extra[:, 128 * t:128 * (t + 1)], 0.0)
                z = _dot(lhs * inv[t], w)
                y = z if y is None else y + z
                pace.before_vpu(0, y[:, -128:] if gl else y[:, :128], k_m)
                yield
            put(y)

        def layer(ps, x):
            d, r = _ln(x)
            xn_s[:, pl.ds(0, D)] = d
            xn_s[:, pl.ds(D, 128)] = r * (DH ** -0.5)

            free = _Pace()
            q = []
            _run(stage_a(0, free, q))
            spread(q[0], 0, free)
            spread(q[0], 1, free)
            _run(stage_a(1, free, q), stage_b(0, 0, free), stage_b(0, 1, free))
            spread(q[1], 0, free)
            spread(q[1], 1, free)
            acc_s[...] = jnp.zeros(acc_s.shape, f32)
            e_s[...] = jnp.ones(e_s.shape, f32)
            y_s[...] = jnp.zeros(y_s.shape, f32)

            def load(i):
                @pl.when(i + look + 1 < NP)
                def _():
                    cp_kv(k_hbm, kb, sem_k, i + look + 1).start()

                @pl.when(i + look < NP)
                def _():
                    start_step(i + look)

                @pl.when(i + look == NP)
                def _():
                    for j in range(4):
                        cp_m(j).start()

                @pl.when(i + 1 < NP)
                def _():
                    cp_kv(k_hbm, kb, sem_k, i + 1).wait()

                cp_kv(v_hbm, vb, sem_v, i).wait()
                for c in range(5):
                    cp_o(i, c).wait()
                flip(i, jnp.where((i & 1) == 0, mt, mtb))
                widen(i)

            def compute(n):
                off = n >> 8

                def to_mxu(slot, val):
                    z_s[1 - off, pl.ds(8 * slot, 8), :] = val

                def to_vpu(slot, val):
                    vb[H * RT - off, pl.ds(8 * slot, 8), :] = pltpu.bitcast(val, u32)

                pace = _Pace(to_mxu, to_vpu, z_s)
                prs, os, scored = {}, {}, {0}

                def vpu_part(u):
                    assert u in scored
                    o = None if sm_first else stage_d1()
                    prs[u] = [p_s[...], softmax(s_s[...], 1, pace, k_sm1)]
                    os[u] = o = o or stage_d1()
                    for t in range(3):
                        pace.before_vpu(("o", t), o[0][t], k_fold + dk_fold * t)
                    yield from stage_c(n * unroll + u, prs[u], pace, mts[u])

                def mxu_part(u):
                    i = n * unroll + u

                    def fin(y):
                        y_s[...] += y if u else jnp.where(i > 0, y, 0.0)

                    q = []
                    pn = jnp.minimum(i + 1, NP - 1)
                    for k in order:
                        if k in "01":
                            yield from stage_b(pn, int(k), pace, lambda: u in prs)
                        elif k == "a":
                            yield from stage_a(jnp.minimum(i + 2, NP - 1), pace, q)
                        elif k == "d":
                            yield from stage_d2(jnp.maximum(i - 1, 0), os[u], pace, fin)
                        elif k == "e":
                            yield from stage_e(i, prs[u], pace, mts[u])
                        else:
                            spread(q[0], "xy".index(k), pace)
                    scored.add(u + 1)

                mxu = _chain(*[mxu_part(u) for u in range(unroll)])
                vpu = _chain(*[vpu_part(u) for u in range(unroll)])
                nm, nc = 32 * unroll + sum(mts), sum(RT * (NT - m) for m in mts)
                done = e = 0
                while done < nc:
                    next(mxu, None)
                    e += 1
                    while done < min(nc, int(e * nc / (nm + lag))):
                        next(vpu, None)
                        done += 1
                    pace.tick(e < nm and e % ez == 0, e % ev == 0)
                _run(mxu, vpu)

            def step(n, carry):
                if dma:
                    @pl.loop(ps * unroll, unroll)
                    def _(u):
                        load(n * unroll + u)
                compute(n)
                return carry

            lax.fori_loop(0, nit // unroll, step, 0)

            def finish(x, wait):
                y = []
                _run(stage_d2(NP - 1, stage_d1(), free, y.append))
                x = x + jnp.sum(y_s[...] + y[0], axis=0, keepdims=True)
                d, r = _ln(x)
                h = []
                if wait:
                    cp_m(0).wait()
                    cp_m(1).wait()
                for c in range(0, F, gw):
                    w = jnp.concatenate([wg[:, pl.ds(c, gw)], wu[:, pl.ds(c, gw)]], axis=1)
                    gu = _dot(d, w) * _wide(r, 2 * gw // 128)
                    h.append((1.0 / (1.0 + jnp.exp(-gu[:, :gw]))) * gu[:, gw:])
                h = jnp.concatenate(h, axis=1)
                if wait:
                    cp_m(2).wait()
                x = x + _dot(h[:, :F - fl], wd[pl.ds(0, F - fl), :])
                if wait:
                    cp_m(3).wait()
                return x + _dot(h[:, F - fl:], wd[pl.ds(F - fl, fl), :])

            if dma:
                return lax.cond(ps == 0, lambda x: finish(x, True), lambda x: finish(x, False), x)
            return finish(x, False)

        if dma:
            for t in range(3 * NP):
                cp_q(t).wait()
            cp_kv(k_hbm, kb, sem_k, 0).wait()
        x = lax.fori_loop(0, npass, layer, x0)
        o_ref[...] = x[:1].astype(o_ref.dtype)

    @jax.jit
    def fn(A_x, A_k_cache, A_v_cache, A_wq, A_wo, B_x, B_w_gate, B_w_up, B_w_down):
        del B_x
        kt = _raw(jnp.swapaxes(A_k_cache, 2, 3).reshape(H * DH, SK))
        vt = _raw(jnp.swapaxes(A_v_cache, 2, 3).reshape(H * DH, SK))
        hbm = pl.BlockSpec(memory_space=pltpu.HBM)
        out = pl.pallas_call(
            kernel,
            out_shape=jax.ShapeDtypeStruct((1, D), bf16),
            in_specs=[hbm] * 8,
            out_specs=pl.BlockSpec(memory_space=pltpu.VMEM),
            scratch_shapes=[
                pltpu.VMEM((H * RT, W // 32, 128), u32),
                pltpu.VMEM((H * RT + 1 + NP * 3 * nu, W // 32, 128), u32),
                pltpu.VMEM((3 * NP, D // 2, 128), u32),
                pltpu.VMEM((5 * NP, DH, 128), u32),
                pltpu.VMEM((D, F), bf16),
                pltpu.VMEM((D, F), bf16),
                pltpu.VMEM((F, D), bf16),
                pltpu.VMEM((24, 8, 128), f32),
                pltpu.VMEM((8, 512), f32),
                pltpu.VMEM((8, 512), f32),
                pltpu.VMEM((2 * NT, 8, 128), f32),
                pltpu.VMEM((2 * RT, 8, 128), f32),
                pltpu.VMEM((2, NZ * 8, 128), f32),
                pltpu.VMEM((8, 1024), f32),
                pltpu.VMEM((8, D + 384), f32),
                pltpu.VMEM((8, D), f32),
                pltpu.VMEM((1, 2 * D), bf16),
                pltpu.SemaphoreType.DMA((1,)),
                pltpu.SemaphoreType.DMA((1,)),
                pltpu.SemaphoreType.DMA((NP,)),
                pltpu.SemaphoreType.DMA((NP,)),
                pltpu.SemaphoreType.DMA((NP,)),
                pltpu.SemaphoreType.DMA((4,)),
            ],
            compiler_params=pltpu.CompilerParams(
                vmem_limit_bytes=int(vm * 1024 * 1024), disable_semaphore_checks=True, flags=flags),
        )(A_x.reshape(1, D), kt, vt, A_wq, A_wo, B_w_gate, B_w_up, B_w_down)
        return out.reshape(1, 1, D)

    return fn


_fn = make(**{'chunk': 6, 'dk_fold': 2, 'gl': False, 'jg': 8, 'k_acc': 1, 'k_fold': 14, 'k_m': 6, 'k_q': 20, 'k_self': 3, 'k_sm': 14, 'k_sm1': 8, 'lag': 4.5, 'look': 2, 'mt': 4, 'mtb': 2, 'order': '0ax1yed', 'sk': 1, 'sm_first': False, 'ucols': [1, 6, 11], 'unroll': 2})


@jax.jit
def pallas_interleave_layers__sliding_block_cached__glu_gated_glu__decode_kernel(
    A_x, A_k_cache, A_v_cache, A_wq, A_wo, B_x, B_w_gate, B_w_up, B_w_down
):
    return _fn(A_x, A_k_cache, A_v_cache, A_wq, A_wo, B_x, B_w_gate, B_w_up, B_w_down)
```

```python
import jax
import jax.numpy as jnp
from jax import lax
import jax.experimental.pallas as pl
import jax.experimental.pallas.tpu as pltpu

H, DH, SK, D, F = 32, 192, 32768, 640, 1536
W = min(4096, max(256, SK // 4))
EPS = 1e-5
NP = H // 2
RT = DH // 8
NT = W // 128
LAYERS = 2
UNROLL = 2
MT = (4, 2)
NU = 3
LOOK = 2
CUTS = (0, 1152, 1408, F)
NZ = 16
bf16, f32, u32 = jnp.bfloat16, jnp.float32, jnp.uint32


def _tiles(a):
    r, c = a.shape
    a = a.reshape(r // 8, 8, c // 128, 128).transpose(0, 2, 1, 3)
    return a.reshape(r // 8, c // 128 * 8, 128)


def _layernorm(x):
    d = x - jnp.sum(x, axis=-1, keepdims=True) * (1.0 / D)
    v = jnp.sum(d * d, axis=-1, keepdims=True) * (1.0 / D)
    return d, jnp.broadcast_to(lax.rsqrt(v + EPS), (8, 128))


def _wide(x, n):
    return jnp.concatenate([x] * n, axis=1)


def _b(x):
    return pltpu.bitcast(x, bf16)


def _dot(a, b):
    return lax.dot_general(a, b, (((1,), (0,)), ((), ())), preferred_element_type=f32)


def _iota(axis):
    return lax.broadcasted_iota(jnp.int32, (8, 128), axis)


def _run(*gens):
    for g in gens:
        for _ in g:
            pass


def _chain(*gens):
    for g in gens:
        yield from g


class _Pace:
    def __init__(self, to_mxu=None, to_vpu=None, z_ref=None):
        self.put, self.z_ref = (to_mxu, to_vpu), z_ref
        self.now, self.due, self.slot = 0, ({}, {}), [0, 0]

    def before_mxu(self, key, val, delay):
        self.due[0][key, self.now] = (self.now + delay, val)

    def before_vpu(self, key, val, delay):
        self.due[1][key, self.now] = (self.now + delay, val)

    def tick(self, mxu):
        self.now += 1
        for w in (0, 1) if mxu else (1,):
            due = self.due[w]
            for key in [k for k, (t, _) in due.items() if t <= self.now]:
                self.slot[w] = (self.slot[w] + 1) % NZ
                self.put[w](self.slot[w], due.pop(key)[1])

    def zero(self):
        if self.z_ref is None:
            return jnp.zeros((8, 128), f32)
        return self.z_ref[0, pl.ds(0, 8), :]


K_MXU, K_ACC, K_SELF, K_SM0, K_SM1, K_FOLD, LAG = 6, 1, 3, 14, 8, 14, 4.5
M_STEPS = sum(5 + 24 + 3 + mt for mt in MT)
V_STEPS = sum(RT * (NT - mt) for mt in MT)


def _kernel(x_hbm, k_hbm, v_hbm, wq_hbm, wo_hbm, wg_hbm, wu_hbm, wd_hbm, o_ref,
            kb, vb, wq, wo, wg, wu, wd, q_s, s_s, p_s, pb_s, acc_s, z_s, e_s, xn_s, y_s, xb,
            sem_x, sem_q, sem_k, sem_v, sem_o, sem_m):
    k_hbm, v_hbm, wq_hbm, wo_hbm = (r.bitcast(u32) for r in (k_hbm, v_hbm, wq_hbm, wo_hbm))

    def cp_x():
        return pltpu.make_async_copy(x_hbm, xb.at[:, pl.ds(0, D)], sem_x.at[0])

    def cp_q(t):
        return pltpu.make_async_copy(wq_hbm.at[:, pl.ds(128 * t, 128)], wq.at[t], sem_q.at[0])

    def cp_kv(hbm, buf, sem, p):
        rows = pl.ds(p * (2 * RT), 2 * RT)
        return pltpu.make_async_copy(
            hbm.at[rows, pl.ds((SK - W) // 32, W // 32)], buf.at[rows], sem.at[p])

    def cp_o(p, c):
        r0 = pl.multiple_of(p * DH, 64)
        return pltpu.make_async_copy(
            wo_hbm.at[pl.ds(r0, DH), pl.ds(128 * c, 128)], wo.at[p * 5 + c], sem_o.at[p])

    def cp_m(j):
        if j < 2:
            return pltpu.make_async_copy((wg_hbm, wu_hbm)[j], (wg, wu)[j], sem_m.at[j])
        rows = pl.ds(CUTS[j - 2], CUTS[j - 1] - CUTS[j - 2])
        return pltpu.make_async_copy(wd_hbm.at[rows], wd.at[rows], sem_m.at[j])

    def start_vo(p):
        cp_kv(v_hbm, vb, sem_v, p).start()
        for c in range(5):
            cp_o(p, c).start()

    cp_x().start()
    for t in range(3 * NP):
        cp_q(t).start()
    cp_kv(k_hbm, kb, sem_k, 0).start()
    for p in range(LOOK):
        cp_kv(k_hbm, kb, sem_k, p + 1).start()
        start_vo(p)
    cp_x().wait()
    z_s[0, pl.ds(0, 8), :] = jnp.zeros((8, 128), f32)
    x0 = jnp.broadcast_to(xb[:, pl.ds(0, D)].astype(f32), (8, D))

    def project(p, pace, out):
        q = None
        for k in range(5):
            w = jnp.concatenate([_b(wq[3 * p + t, pl.ds(64 * k, 64), :]) for t in range(3)], axis=1)
            t = _dot(xn_s[:, pl.ds(128 * k, 128)] + pace.zero(), w)
            q = t if q is None else q + t
            pace.before_vpu(0, q[:, :128], K_MXU)
            yield
        out.append(q * _wide(xn_s[:, pl.ds(D, 128)], 3))

    def spread(q, a):
        lane = _iota(1)
        for g in range(12 * a, 12 * a + 12):
            qt = q[:, 128 * (g // 8):128 * (g // 8 + 1)]
            q_s[g] = jnp.take_along_axis(qt, ((lane >> 6) << 3) + (lane & 7) + 16 * (g % 8), axis=1)

    def scores(p, a, pace, consumed=lambda: True):
        diag = ((_iota(1) >> 3) & 7) == _iota(0)
        s = None
        for kt in range(12):
            lhs = jnp.where(diag, q_s[12 * a + kt], pace.zero())
            r0 = p * (2 * RT) + a * RT + 2 * kt
            rhs = jnp.concatenate(
                [_b(kb[pl.ds(r0, 2), pl.ds(32 * c, 32), :].reshape(64, 128)) for c in range(4)],
                axis=1)
            t = _dot(lhs, rhs)
            s = t if s is None else s + t
            pace.before_vpu(0, s[:, :128], K_MXU)
            yield
        assert consumed()
        if a == 1:
            s_s[...] = s
        else:
            p_s[...] = softmax_numerator(s, a, pace, K_SM0)

    def softmax_numerator(s, a, pace, delay):
        m = jnp.max(jnp.max(s, axis=1, keepdims=True), axis=0, keepdims=True)
        e = jnp.exp(s - m)
        pace.before_vpu(("sm", a), e[:, :128], delay)
        return e

    def row(pr, t):
        return jnp.broadcast_to(pr[t % 8:t % 8 + 1, 128 * (t // 8):128 * (t // 8 + 1)], (8, 128))

    def upper(p, rt, j):
        k = rt * NU + j
        return H * RT + 1 + p * (3 * NU) + k // 16, pl.ds(8 * (k % 16), 8), slice(None)

    def widen(p):
        for r in range(0, 2 * RT, 8):
            vs = {(rt, j): _b(vb[p * (2 * RT) + rt, pl.ds(8 * j, 8), :]).astype(f32)
                  for rt in range(r, r + 8) for j in range(NU)}
            for (rt, j), v in vs.items():
                vb[p * (2 * RT) + rt, pl.ds(8 * j, 8), :] = pltpu.bitcast(v[:8], u32)
                vb[upper(p, rt, j)] = pltpu.bitcast(v[8:], u32)

    def flip(p, mt):
        @pl.loop((NT - mt) // 2, NT // 2)
        def _(j):
            cols = pl.ds(pl.multiple_of(8 * j, 8), 8)
            vs = [_b(vb[pl.ds(p * (2 * RT) + 16 * u, 16), cols, :]).astype(f32) for u in range(3)]
            ts = [v[:, 8 * h:8 * h + 8, :].reshape(128, 128).T.astype(bf16)
                  for v in vs for h in range(2)]
            for n, t in enumerate(ts):
                vb[pl.ds(p * (2 * RT) + 8 * n, 8), cols, :] = (
                    pltpu.bitcast(t, u32).reshape(8, 8, 128))

    def pv_vpu(p, prs, pace, mt):
        nv = (NT - mt) // 2
        for a in range(2):
            e = [prs[a][:, 128 * c:128 * (c + 1)] for c in range(4)]
            e_s[:, pl.ds(384 + 128 * a, 128)] = (e[0] + e[1]) + (e[2] + e[3])
            have = []
            for r in range(a * RT, (a + 1) * RT, 6):
                acc = [None] * 6
                for n, i in [(n, i) for i0 in range(0, nv, 8) for n in range(6)
                             for i in range(i0, min(i0 + 8, nv))]:
                    j = (i + n) % nv
                    if j not in have:
                        have.append(j)
                        for t in (2 * j, 2 * j + 1):
                            pb_s[NT * a + t] = row(prs[a], t)
                    p0, p1 = pb_s[NT * a + 2 * j], pb_s[NT * a + 2 * j + 1]
                    v = vb[p * (2 * RT) + r + n, pl.ds(8 * j, 8), :]
                    if j < NU:
                        v0, v1 = pltpu.bitcast(v, f32), pltpu.bitcast(vb[upper(p, r + n, j)], f32)
                    else:
                        v = _b(v).astype(f32)
                        v0, v1 = v[:8], v[8:]
                    if acc[n] is None:
                        acc[n] = v0 * p0 + v1 * p1
                    else:
                        acc[n] = (acc[n] + v0 * p0) + v1 * p1
                    pace.before_mxu(r + n, acc[n], K_ACC)
                    if pace.now + K_SELF < K_MXU:
                        pace.before_vpu("self", acc[n], K_SELF)
                    yield
                for n in range(6):
                    acc_s[r + n] = acc[n]

    def pv_mxu(p, prs, pace, mt):
        o = None
        for t in range(NT - mt, NT):
            lhs = jnp.where(_iota(0) < 4, row(prs[0], t), row(prs[1], t)) + pace.zero()
            r0 = p * (2 * RT) + 8 * (t % 2)
            w = jnp.concatenate(
                [_b(vb[pl.ds(r0 + 16 * u, 8), pl.ds(8 * (t // 2), 8), :].reshape(64, 128))
                 for u in range(3)], axis=1)
            z = _dot(lhs, w)
            o = z if o is None else o + z
            pace.before_vpu(0, o[:, :128], K_MXU)
            yield
        e_s[:, pl.ds(0, 384)] = o

    def fold():
        def merge(lo, n):
            if n == 1:
                return jnp.broadcast_to(jnp.sum(acc_s[lo], axis=1, keepdims=True), (8, 128))
            n //= 2
            return jnp.where((_iota(1) & (8 * n)) == 0, merge(lo, n), merge(lo + n, n))

        tiles = [merge(16 * t, 16) for t in range(3)]
        inv = []
        for a in range(2):
            l = jnp.sum(e_s[:, pl.ds(384 + 128 * a, 128)], axis=0, keepdims=True)
            inv.append(jnp.broadcast_to(1.0 / jnp.sum(l, axis=1, keepdims=True), (8, 128)))
        inv = [inv[0], jnp.where(_iota(1) < 64, inv[0], inv[1]), inv[1]]
        return tiles, e_s[:, pl.ds(0, 384)], inv

    def out_project(p, o, pace, put):
        tiles, extra, inv = o
        y = None
        lane, sub = _iota(1), _iota(0)
        for t in range(3):
            w = jnp.concatenate([_b(wo[5 * p + c, pl.ds(64 * t, 64), :]) for c in range(5)], axis=1)
            lhs = jnp.where((lane & 7) == sub, tiles[t], pace.zero())
            pick = sub == (0, (lane >> 6) << 2, 4)[t]
            lhs = lhs + jnp.where(pick, extra[:, 128 * t:128 * (t + 1)], 0.0)
            z = _dot(lhs * inv[t], w)
            y = z if y is None else y + z
            pace.before_vpu(0, y[:, :128], K_MXU)
            yield
        put(y)

    def load(i):
        @pl.when(i + LOOK + 1 < NP)
        def _():
            cp_kv(k_hbm, kb, sem_k, i + LOOK + 1).start()

        @pl.when(i + LOOK < NP)
        def _():
            start_vo(i + LOOK)

        @pl.when(i + LOOK == NP)
        def _():
            for j in range(len(CUTS) + 1):
                cp_m(j).start()

        @pl.when(i + 1 < NP)
        def _():
            cp_kv(k_hbm, kb, sem_k, i + 1).wait()

        cp_kv(v_hbm, vb, sem_v, i).wait()
        for c in range(5):
            cp_o(i, c).wait()
        flip(i, jnp.where((i & 1) == 0, MT[0], MT[1]))
        widen(i)

    def compute(n):
        off = n >> 8

        def to_mxu(slot, val):
            z_s[1 - off, pl.ds(8 * slot, 8), :] = val

        def to_vpu(slot, val):
            vb[H * RT - off, pl.ds(8 * slot, 8), :] = pltpu.bitcast(val, u32)

        pace = _Pace(to_mxu, to_vpu, z_s)
        prs, outs, scored = {}, {}, [0]

        def vpu_part(u):
            assert u in scored
            outs[u] = fold()
            prs[u] = [p_s[...], softmax_numerator(s_s[...], 1, pace, K_SM1)]
            for t in range(3):
                pace.before_vpu(("o", t), outs[u][0][t], K_FOLD + 2 * t)
            yield from pv_vpu(n * UNROLL + u, prs[u], pace, MT[u])

        def mxu_part(u):
            i = n * UNROLL + u

            def add(y):
                y_s[...] += y if u else jnp.where(i > 0, y, 0.0)

            q = []
            nxt = jnp.minimum(i + 1, NP - 1)
            yield from scores(nxt, 0, pace, lambda: u in prs)
            yield from project(jnp.minimum(i + 2, NP - 1), pace, q)
            spread(q[0], 0)
            yield from scores(nxt, 1, pace, lambda: u in prs)
            spread(q[0], 1)
            yield from pv_mxu(i, prs[u], pace, MT[u])
            yield from out_project(jnp.maximum(i - 1, 0), outs[u], pace, add)
            scored.append(u + 1)

        mxu = _chain(*[mxu_part(u) for u in range(UNROLL)])
        vpu = _chain(*[vpu_part(u) for u in range(UNROLL)])
        done = e = 0
        while done < V_STEPS:
            next(mxu, None)
            e += 1
            while done < min(V_STEPS, int(e * V_STEPS / (M_STEPS + LAG))):
                next(vpu, None)
                done += 1
            pace.tick(e < M_STEPS)
        _run(mxu, vpu)

    def finish(x, wait):
        y = []
        _run(out_project(NP - 1, fold(), _Pace(), y.append))
        x = x + jnp.sum(y_s[...] + y[0], axis=0, keepdims=True)
        d, r = _layernorm(x)
        h = []
        if wait:
            cp_m(0).wait()
            cp_m(1).wait()
        for c in range(0, F, 256):
            w = jnp.concatenate([wg[:, pl.ds(c, 256)], wu[:, pl.ds(c, 256)]], axis=1)
            gu = _dot(d, w) * _wide(r, 4)
            h.append((1.0 / (1.0 + jnp.exp(-gu[:, :256]))) * gu[:, 256:])
        h = jnp.concatenate(h, axis=1)
        for j, (lo, hi) in enumerate(zip(CUTS, CUTS[1:])):
            if wait:
                cp_m(2 + j).wait()
            x = x + _dot(h[:, lo:hi], wd[pl.ds(lo, hi - lo), :])
        return x

    def layer(li, x):
        d, r = _layernorm(x)
        xn_s[:, pl.ds(0, D)] = d
        xn_s[:, pl.ds(D, 128)] = r * (DH ** -0.5)

        free = _Pace()
        q = []
        _run(project(0, free, q))
        spread(q[0], 0)
        spread(q[0], 1)
        _run(project(1, free, q), scores(0, 0, free), scores(0, 1, free))
        spread(q[1], 0)
        spread(q[1], 1)
        acc_s[...] = jnp.zeros(acc_s.shape, f32)
        e_s[...] = jnp.ones(e_s.shape, f32)
        y_s[...] = jnp.zeros(y_s.shape, f32)

        def step(n, carry):
            @pl.loop(li * UNROLL, UNROLL)
            def _(u):
                load(n * UNROLL + u)

            compute(n)
            return carry

        lax.fori_loop(0, NP // UNROLL, step, 0)
        return lax.cond(li == 0, lambda x: finish(x, True), lambda x: finish(x, False), x)

    for t in range(3 * NP):
        cp_q(t).wait()
    cp_kv(k_hbm, kb, sem_k, 0).wait()
    x = lax.fori_loop(0, LAYERS, layer, x0)
    o_ref[...] = x[:1].astype(o_ref.dtype)


@jax.jit
def pallas_interleave_layers__sliding_block_cached__glu_gated_glu__decode_kernel(
    A_x: jax.Array,
    A_k_cache: jax.Array,
    A_v_cache: jax.Array,
    A_wq: jax.Array,
    A_wo: jax.Array,
    B_x: jax.Array,
    B_w_gate: jax.Array,
    B_w_up: jax.Array,
    B_w_down: jax.Array,
):
    del B_x
    assert A_k_cache.shape == A_v_cache.shape == (1, H, SK, DH)
    kt = _tiles(jnp.swapaxes(A_k_cache, 2, 3).reshape(H * DH, SK))
    vt = _tiles(jnp.swapaxes(A_v_cache, 2, 3).reshape(H * DH, SK))
    out = pl.pallas_call(
        _kernel,
        out_shape=jax.ShapeDtypeStruct((1, D), A_x.dtype),
        in_specs=[pl.BlockSpec(memory_space=pltpu.HBM)] * 8,
        out_specs=pl.BlockSpec(memory_space=pltpu.VMEM),
        scratch_shapes=[
            pltpu.VMEM((H * RT, W // 32, 128), u32),
            pltpu.VMEM((H * RT + 1 + NP * 3 * NU, W // 32, 128), u32),
            pltpu.VMEM((3 * NP, D // 2, 128), u32),
            pltpu.VMEM((5 * NP, DH, 128), u32),
            pltpu.VMEM((D, F), bf16),
            pltpu.VMEM((D, F), bf16),
            pltpu.VMEM((F, D), bf16),
            pltpu.VMEM((24, 8, 128), f32),
            pltpu.VMEM((8, 512), f32),
            pltpu.VMEM((8, 512), f32),
            pltpu.VMEM((2 * NT, 8, 128), f32),
            pltpu.VMEM((2 * RT, 8, 128), f32),
            pltpu.VMEM((2, NZ * 8, 128), f32),
            pltpu.VMEM((8, 1024), f32),
            pltpu.VMEM((8, D + 384), f32),
            pltpu.VMEM((8, D), f32),
            pltpu.VMEM((1, 2 * D), bf16),
            pltpu.SemaphoreType.DMA((1,)),
            pltpu.SemaphoreType.DMA((1,)),
            pltpu.SemaphoreType.DMA((NP,)),
            pltpu.SemaphoreType.DMA((NP,)),
            pltpu.SemaphoreType.DMA((NP,)),
            pltpu.SemaphoreType.DMA((len(CUTS) + 1,)),
        ],
        compiler_params=pltpu.CompilerParams(
            vmem_limit_bytes=127 * 1024 * 1024, disable_semaphore_checks=True),
    )(A_x.reshape(1, D), kt, vt, A_wq, A_wo, B_w_gate, B_w_up, B_w_down)
    return out.reshape(1, 1, D)
```

```python
import jax
import jax.numpy as jnp
from jax import lax
import jax.experimental.pallas as pl
import jax.experimental.pallas.tpu as pltpu

H, DH, SK, D, F = 32, 192, 32768, 640, 1536
W = min(4096, max(256, SK // 4))
EPS = 1e-5
NP = H // 2
RT = DH // 8
NT = W // 128
LAYERS = 2
UNROLL = 2
MT = (4, 2)
NU = 3
LOOK = 2
KV = (0, 1, 1, 1, 2, 2)
CUTS = (0, 1152, 1408, F)
NZ = 16
bf16, f32, u32 = jnp.bfloat16, jnp.float32, jnp.uint32


def _tiles(a):
    r, c = a.shape
    a = a.reshape(r // 8, 8, c // 128, 128).transpose(0, 2, 1, 3)
    return a.reshape(r // 8, c // 128 * 8, 128)


def _layernorm(x):
    d = x - jnp.sum(x, axis=-1, keepdims=True) * (1.0 / D)
    v = jnp.sum(d * d, axis=-1, keepdims=True) * (1.0 / D)
    return d, jnp.broadcast_to(lax.rsqrt(v + EPS), (8, 128))


def _wide(x, n):
    return jnp.concatenate([x] * n, axis=1)


def _b(x):
    return pltpu.bitcast(x, bf16)


def _dot(a, b):
    return lax.dot_general(a, b, (((1,), (0,)), ((), ())), preferred_element_type=f32)


def _iota(axis):
    return lax.broadcasted_iota(jnp.int32, (8, 128), axis)


def _run(*gens):
    for g in gens:
        for _ in g:
            pass


def _chain(*gens):
    for g in gens:
        yield from g


class _Pace:
    def __init__(self, to_mxu=None, to_vpu=None, z_ref=None):
        self.put, self.z_ref = (to_mxu, to_vpu), z_ref
        self.now, self.due, self.slot = 0, ({}, {}), [0, 0]

    def before_mxu(self, key, val, delay):
        self.due[0][key, self.now] = (self.now + delay, val)

    def before_vpu(self, key, val, delay):
        self.due[1][key, self.now] = (self.now + delay, val)

    def tick(self, mxu):
        self.now += 1
        for w in (0, 1) if mxu else (1,):
            due = self.due[w]
            for key in [k for k, (t, _) in due.items() if t <= self.now]:
                self.slot[w] = (self.slot[w] + 1) % NZ
                self.put[w](self.slot[w], due.pop(key)[1])

    def zero(self):
        if self.z_ref is None:
            return jnp.zeros((8, 128), f32)
        return self.z_ref[0, pl.ds(0, 8), :]


K_MXU, K_ACC, K_SELF, K_SM0, K_SM1, K_FOLD, LAG = 6, 1, 3, 14, 8, 14, 4.5
M_STEPS = sum(5 + 24 + 3 + mt for mt in MT)
V_STEPS = sum(RT * (NT - mt) for mt in MT)


def _kernel(x_hbm, k_hbm, v_hbm, wq_hbm, wo_hbm, wg_hbm, wu_hbm, wd_hbm, o_ref,
            kb, vb, wq, wo, wg, wu, wd, q_s, s_s, p_s, pb_s, acc_s, z_s, e_s, xn_s, y_s, xb,
            sem_x, sem_q, sem_k, sem_v, sem_o, sem_m):
    k_hbm, v_hbm, wq_hbm, wo_hbm = (r.bitcast(u32) for r in (k_hbm, v_hbm, wq_hbm, wo_hbm))

    def cp_x():
        return pltpu.make_async_copy(x_hbm, xb.at[:, pl.ds(0, D)], sem_x.at[0])

    def cp_q(t):
        return pltpu.make_async_copy(wq_hbm.at[:, pl.ds(128 * t, 128)], wq.at[t], sem_q.at[0])

    def cp_kv(hbm, buf, sem, p):
        rows = pl.ds(p * (2 * RT), 2 * RT)
        return pltpu.make_async_copy(
            hbm.at[rows, pl.ds((SK - W) // 32, W // 32)], buf.at[rows], sem.at[p])

    def cp_o(p, c):
        r0 = pl.multiple_of(p * DH, 64)
        return pltpu.make_async_copy(
            wo_hbm.at[pl.ds(r0, DH), pl.ds(128 * c, 128)], wo.at[p * 5 + c], sem_o.at[p])

    def cp_m(j):
        if j < 2:
            return pltpu.make_async_copy((wg_hbm, wu_hbm)[j], (wg, wu)[j], sem_m.at[j])
        rows = pl.ds(CUTS[j - 2], CUTS[j - 1] - CUTS[j - 2])
        return pltpu.make_async_copy(wd_hbm.at[rows], wd.at[rows], sem_m.at[j])

    def start_vo(p):
        cp_kv(v_hbm, vb, sem_v, p).start()
        for c in range(5):
            cp_o(p, c).start()

    cp_x().start()
    for t in range(3 * NP):
        cp_q(t).start()
    cp_kv(k_hbm, kb, sem_k, 0).start()
    for p in range(LOOK):
        cp_kv(k_hbm, kb, sem_k, p + 1).start()
        start_vo(p)
    cp_x().wait()
    z_s[0, pl.ds(0, 8), :] = jnp.zeros((8, 128), f32)
    x0 = jnp.broadcast_to(xb[:, pl.ds(0, D)].astype(f32), (8, D))

    def project(p, pace, out):
        q = None
        for k in range(5):
            w = jnp.concatenate([_b(wq[3 * p + t, pl.ds(64 * k, 64), :]) for t in range(3)], axis=1)
            t = _dot(xn_s[:, pl.ds(128 * k, 128)] + pace.zero(), w)
            q = t if q is None else q + t
            pace.before_vpu(0, q[:, :128], K_MXU)
            yield
        out.append(q * _wide(xn_s[:, pl.ds(D, 128)], 3))

    def spread(q, a):
        lane = _iota(1)
        for g in range(12 * a, 12 * a + 12):
            qt = q[:, 128 * (g // 8):128 * (g // 8 + 1)]
            q_s[g] = jnp.take_along_axis(qt, ((lane >> 6) << 3) + (lane & 7) + 16 * (g % 8), axis=1)

    def scores(p, a, pace, consumed=lambda: True):
        diag = ((_iota(1) >> 3) & 7) == _iota(0)
        s = None
        for kt in range(12):
            lhs = jnp.where(diag, q_s[12 * a + kt], pace.zero())
            r0 = p * (2 * RT) + a * RT + 2 * kt
            rhs = jnp.concatenate(
                [_b(kb[pl.ds(r0, 2), pl.ds(32 * c, 32), :].reshape(64, 128)) for c in range(4)],
                axis=1)
            t = _dot(lhs, rhs)
            s = t if s is None else s + t
            pace.before_vpu(0, s[:, :128], K_MXU)
            yield
        assert consumed()
        if a == 1:
            s_s[...] = s
        else:
            p_s[...] = softmax_numerator(s, a, pace, K_SM0)

    def softmax_numerator(s, a, pace, delay):
        m = jnp.max(jnp.max(s, axis=1, keepdims=True), axis=0, keepdims=True)
        e = jnp.exp(s - m)
        pace.before_vpu(("sm", a), e[:, :128], delay)
        return e

    def row(pr, t):
        return jnp.broadcast_to(pr[t % 8:t % 8 + 1, 128 * (t // 8):128 * (t // 8 + 1)], (8, 128))

    def upper(p, rt, j):
        k = rt * NU + j
        return H * RT + 1 + p * (3 * NU) + k // 16, pl.ds(8 * (k % 16), 8), slice(None)

    def widen(p):
        for r in range(0, 2 * RT, 8):
            vs = {(rt, j): _b(vb[p * (2 * RT) + rt, pl.ds(8 * j, 8), :]).astype(f32)
                  for rt in range(r, r + 8) for j in range(NU)}
            for (rt, j), v in vs.items():
                vb[p * (2 * RT) + rt, pl.ds(8 * j, 8), :] = pltpu.bitcast(v[:8], u32)
                vb[upper(p, rt, j)] = pltpu.bitcast(v[8:], u32)

    def flip(p, mt):
        @pl.loop((NT - mt) // 2, NT // 2)
        def _(j):
            cols = pl.ds(pl.multiple_of(8 * j, 8), 8)
            vs = [_b(vb[pl.ds(p * (2 * RT) + 16 * u, 16), cols, :]).astype(f32) for u in range(3)]
            ts = [v[:, 8 * h:8 * h + 8, :].reshape(128, 128).T.astype(bf16)
                  for v in vs for h in range(2)]
            for n, t in enumerate(ts):
                vb[pl.ds(p * (2 * RT) + 8 * n, 8), cols, :] = (
                    pltpu.bitcast(t, u32).reshape(8, 8, 128))

    def pv_vpu(p, prs, pace, mt):
        nv = (NT - mt) // 2
        for a in range(2):
            e = [prs[a][:, 128 * c:128 * (c + 1)] for c in range(4)]
            e_s[:, pl.ds(384 + 128 * a, 128)] = (e[0] + e[1]) + (e[2] + e[3])
            have = []
            for r in range(a * RT, (a + 1) * RT, 6):
                acc = [None] * 6
                for n, i in [(n, i) for i0 in range(0, nv, 8) for n in range(6)
                             for i in range(i0, min(i0 + 8, nv))]:
                    j = (i + n) % nv
                    if j not in have:
                        have.append(j)
                        for t in (2 * j, 2 * j + 1):
                            pb_s[NT * a + t] = row(prs[a], t)
                    p0, p1 = pb_s[NT * a + 2 * j], pb_s[NT * a + 2 * j + 1]
                    v = vb[p * (2 * RT) + r + n, pl.ds(8 * j, 8), :]
                    if j < NU:
                        v0, v1 = pltpu.bitcast(v, f32), pltpu.bitcast(vb[upper(p, r + n, j)], f32)
                    else:
                        v = _b(v).astype(f32)
                        v0, v1 = v[:8], v[8:]
                    if acc[n] is None:
                        acc[n] = v0 * p0 + v1 * p1
                    else:
                        acc[n] = (acc[n] + v0 * p0) + v1 * p1
                    pace.before_mxu(r + n, acc[n], K_ACC)
                    if pace.now + K_SELF < K_MXU:
                        pace.before_vpu("self", acc[n], K_SELF)
                    yield
                for n in range(6):
                    acc_s[r + n] = acc[n]

    def pv_mxu(p, prs, pace, mt):
        o = None
        for t in range(NT - mt, NT):
            lhs = jnp.where(_iota(0) < 4, row(prs[0], t), row(prs[1], t)) + pace.zero()
            r0 = p * (2 * RT) + 8 * (t % 2)
            w = jnp.concatenate(
                [_b(vb[pl.ds(r0 + 16 * u, 8), pl.ds(8 * (t // 2), 8), :].reshape(64, 128))
                 for u in range(3)], axis=1)
            z = _dot(lhs, w)
            o = z if o is None else o + z
            pace.before_vpu(0, o[:, :128], K_MXU)
            yield
        e_s[:, pl.ds(0, 384)] = o

    def fold():
        def merge(lo, n):
            if n == 1:
                return jnp.broadcast_to(jnp.sum(acc_s[lo], axis=1, keepdims=True), (8, 128))
            n //= 2
            return jnp.where((_iota(1) & (8 * n)) == 0, merge(lo, n), merge(lo + n, n))

        tiles = [merge(16 * t, 16) for t in range(3)]
        inv = []
        for a in range(2):
            l = jnp.sum(e_s[:, pl.ds(384 + 128 * a, 128)], axis=0, keepdims=True)
            inv.append(jnp.broadcast_to(1.0 / jnp.sum(l, axis=1, keepdims=True), (8, 128)))
        inv = [inv[0], jnp.where(_iota(1) < 64, inv[0], inv[1]), inv[1]]
        return tiles, e_s[:, pl.ds(0, 384)], inv

    def out_project(p, o, pace, put):
        tiles, extra, inv = o
        y = None
        lane, sub = _iota(1), _iota(0)
        for t in range(3):
            w = jnp.concatenate([_b(wo[5 * p + c, pl.ds(64 * t, 64), :]) for c in range(5)], axis=1)
            lhs = jnp.where((lane & 7) == sub, tiles[t], pace.zero())
            pick = sub == (0, (lane >> 6) << 2, 4)[t]
            lhs = lhs + jnp.where(pick, extra[:, 128 * t:128 * (t + 1)], 0.0)
            z = _dot(lhs * inv[t], w)
            y = z if y is None else y + z
            pace.before_vpu(0, y[:, :128], K_MXU)
            yield
        put(y)

    def load(i):
        @pl.when(i + LOOK + 1 < NP)
        def _():
            cp_kv(k_hbm, kb, sem_k, i + LOOK + 1).start()

        @pl.when(i + LOOK < NP)
        def _():
            start_vo(i + LOOK)

        @pl.when(i + LOOK == NP)
        def _():
            for j in range(len(CUTS) + 1):
                cp_m(j).start()

        @pl.when(i + 1 < NP)
        def _():
            cp_kv(k_hbm, kb, sem_k, i + 1).wait()

        cp_kv(v_hbm, vb, sem_v, i).wait()
        for c in range(5):
            cp_o(i, c).wait()
        flip(i, jnp.where((i & 1) == 0, MT[0], MT[1]))
        widen(i)

    def compute(n):
        off = n >> 8

        def to_mxu(slot, val):
            z_s[1 - off, pl.ds(8 * slot, 8), :] = val

        def to_vpu(slot, val):
            vb[H * RT - off, pl.ds(8 * slot, 8), :] = pltpu.bitcast(val, u32)

        pace = _Pace(to_mxu, to_vpu, z_s)
        prs, outs, scored = {}, {}, [0]

        def vpu_part(u):
            assert u in scored
            outs[u] = fold()
            prs[u] = [p_s[...], softmax_numerator(s_s[...], 1, pace, K_SM1)]
            for t in range(3):
                pace.before_vpu(("o", t), outs[u][0][t], K_FOLD + 2 * t)
            yield from pv_vpu(n * UNROLL + u, prs[u], pace, MT[u])

        def mxu_part(u):
            i = n * UNROLL + u

            def add(y):
                y_s[...] += y if u else jnp.where(i > 0, y, 0.0)

            q = []
            nxt = jnp.minimum(i + 1, NP - 1)
            yield from scores(nxt, 0, pace, lambda: u in prs)
            yield from project(jnp.minimum(i + 2, NP - 1), pace, q)
            spread(q[0], 0)
            yield from scores(nxt, 1, pace, lambda: u in prs)
            spread(q[0], 1)
            yield from pv_mxu(i, prs[u], pace, MT[u])
            yield from out_project(jnp.maximum(i - 1, 0), outs[u], pace, add)
            scored.append(u + 1)

        mxu = _chain(*[mxu_part(u) for u in range(UNROLL)])
        vpu = _chain(*[vpu_part(u) for u in range(UNROLL)])
        done = e = 0
        while done < V_STEPS:
            next(mxu, None)
            e += 1
            while done < min(V_STEPS, int(e * V_STEPS / (M_STEPS + LAG))):
                next(vpu, None)
                done += 1
            pace.tick(e < M_STEPS)
        _run(mxu, vpu)

    def finish(x, wait):
        y = []
        _run(out_project(NP - 1, fold(), _Pace(), y.append))
        x = x + jnp.sum(y_s[...] + y[0], axis=0, keepdims=True)
        d, r = _layernorm(x)
        h = []
        if wait:
            cp_m(0).wait()
            cp_m(1).wait()
        mean = jnp.sum(x, axis=-1, keepdims=True) * (1.0 / D)
        col = {k: jnp.broadcast_to(x[:1, k:k + 128], (128, 128)).T - mean[:1]
               for k in range(D - 128 * max(KV), D, 128)}
        for c, kv in zip(range(0, F, 256), KV):
            k0 = D - 128 * kv
            w = jnp.concatenate([m[pl.ds(0, k0), pl.ds(c, 256)] for m in (wg, wu)], axis=1)
            gu = _dot(d[:, :k0], w)
            if kv:
                acc = None
                for k in range(k0, D, 8):
                    w = jnp.concatenate(
                        [m[pl.ds(k, 8), pl.ds(c, 256)].astype(f32) for m in (wg, wu)], axis=1)
                    t = w * _wide(col[k // 128 * 128][k % 128:k % 128 + 8], 4)
                    acc = t if acc is None else acc + t
                gu = gu + jnp.sum(acc, axis=0, keepdims=True)
            gu = gu * _wide(r, 4)
            h.append((1.0 / (1.0 + jnp.exp(-gu[:, :256]))) * gu[:, 256:])
        h = jnp.concatenate(h, axis=1)
        for j, (lo, hi) in enumerate(zip(CUTS, CUTS[1:])):
            if wait:
                cp_m(2 + j).wait()
            x = x + _dot(h[:, lo:hi], wd[pl.ds(lo, hi - lo), :])
        return x

    def layer(li, x):
        d, r = _layernorm(x)
        xn_s[:, pl.ds(0, D)] = d
        xn_s[:, pl.ds(D, 128)] = r * (DH ** -0.5)

        free = _Pace()
        q = []
        _run(project(0, free, q))
        spread(q[0], 0)
        spread(q[0], 1)
        _run(project(1, free, q), scores(0, 0, free), scores(0, 1, free))
        spread(q[1], 0)
        spread(q[1], 1)
        acc_s[...] = jnp.zeros(acc_s.shape, f32)
        e_s[...] = jnp.ones(e_s.shape, f32)
        y_s[...] = jnp.zeros(y_s.shape, f32)

        def step(n, carry):
            @pl.loop(li * UNROLL, UNROLL)
            def _(u):
                load(n * UNROLL + u)

            compute(n)
            return carry

        lax.fori_loop(0, NP // UNROLL, step, 0)
        return lax.cond(li == 0, lambda x: finish(x, True), lambda x: finish(x, False), x)

    for t in range(3 * NP):
        cp_q(t).wait()
    cp_kv(k_hbm, kb, sem_k, 0).wait()
    x = lax.fori_loop(0, LAYERS, layer, x0)
    o_ref[...] = x[:1].astype(o_ref.dtype)


@jax.jit
def pallas_interleave_layers__sliding_block_cached__glu_gated_glu__decode_kernel(
    A_x: jax.Array,
    A_k_cache: jax.Array,
    A_v_cache: jax.Array,
    A_wq: jax.Array,
    A_wo: jax.Array,
    B_x: jax.Array,
    B_w_gate: jax.Array,
    B_w_up: jax.Array,
    B_w_down: jax.Array,
):
    del B_x
    assert A_k_cache.shape == A_v_cache.shape == (1, H, SK, DH)
    kt = _tiles(jnp.swapaxes(A_k_cache, 2, 3).reshape(H * DH, SK))
    vt = _tiles(jnp.swapaxes(A_v_cache, 2, 3).reshape(H * DH, SK))
    out = pl.pallas_call(
        _kernel,
        out_shape=jax.ShapeDtypeStruct((1, D), A_x.dtype),
        in_specs=[pl.BlockSpec(memory_space=pltpu.HBM)] * 8,
        out_specs=pl.BlockSpec(memory_space=pltpu.VMEM),
        scratch_shapes=[
            pltpu.VMEM((H * RT, W // 32, 128), u32),
            pltpu.VMEM((H * RT + 1 + NP * 3 * NU, W // 32, 128), u32),
            pltpu.VMEM((3 * NP, D // 2, 128), u32),
            pltpu.VMEM((5 * NP, DH, 128), u32),
            pltpu.VMEM((D, F), bf16),
            pltpu.VMEM((D, F), bf16),
            pltpu.VMEM((F, D), bf16),
            pltpu.VMEM((24, 8, 128), f32),
            pltpu.VMEM((8, 512), f32),
            pltpu.VMEM((8, 512), f32),
            pltpu.VMEM((2 * NT, 8, 128), f32),
            pltpu.VMEM((2 * RT, 8, 128), f32),
            pltpu.VMEM((2, NZ * 8, 128), f32),
            pltpu.VMEM((8, 1024), f32),
            pltpu.VMEM((8, D + 384), f32),
            pltpu.VMEM((8, D), f32),
            pltpu.VMEM((1, 2 * D), bf16),
            pltpu.SemaphoreType.DMA((1,)),
            pltpu.SemaphoreType.DMA((1,)),
            pltpu.SemaphoreType.DMA((NP,)),
            pltpu.SemaphoreType.DMA((NP,)),
            pltpu.SemaphoreType.DMA((NP,)),
            pltpu.SemaphoreType.DMA((len(CUTS) + 1,)),
        ],
        compiler_params=pltpu.CompilerParams(
            vmem_limit_bytes=127 * 1024 * 1024, disable_semaphore_checks=True),
    )(A_x.reshape(1, D), kt, vt, A_wq, A_wo, B_w_gate, B_w_up, B_w_down)
    return out.reshape(1, 1, D)
```

```python
import jax
import jax.numpy as jnp
from jax import lax
import jax.experimental.pallas as pl
import jax.experimental.pallas.tpu as pltpu

H, DH, SK, D, F = 32, 192, 32768, 640, 1536
W = min(4096, max(256, SK // 4))
EPS = 1e-5
NP = H // 2
RT = DH // 8
NT = W // 128
LAYERS = 2
UNROLL = 2
MT = (4, 2)
NU = 3
LOOK = 2
KV = (0, 1, 1, 1, 2, 2)
CUTS = (0, 1152, 1408, F)
NZ = 16
bf16, f32, u32 = jnp.bfloat16, jnp.float32, jnp.uint32


def _tiles(a):
    r, c = a.shape
    a = a.reshape(r // 8, 8, c // 128, 128).transpose(0, 2, 1, 3)
    return a.reshape(r // 8, c // 128 * 8, 128)


def _layernorm(x):
    d = x - jnp.sum(x, axis=-1, keepdims=True) * (1.0 / D)
    v = jnp.sum(d * d, axis=-1, keepdims=True) * (1.0 / D)
    return d, jnp.broadcast_to(lax.rsqrt(v + EPS), (8, 128))


def _wide(x, n):
    return jnp.concatenate([x] * n, axis=1)


def _b(x):
    return pltpu.bitcast(x, bf16)


def _dot(a, b):
    return lax.dot_general(a, b, (((1,), (0,)), ((), ())), preferred_element_type=f32)


def _iota(axis):
    return lax.broadcasted_iota(jnp.int32, (8, 128), axis)


def _run(*gens):
    for g in gens:
        for _ in g:
            pass


def _chain(*gens):
    for g in gens:
        yield from g


class _Pace:
    def __init__(self, to_mxu=None, to_vpu=None, z_ref=None):
        self.put, self.z_ref = (to_mxu, to_vpu), z_ref
        self.now, self.due, self.slot = 0, ({}, {}), [0, 0]

    def before_mxu(self, key, val, delay):
        self.due[0][key, self.now] = (self.now + delay, val)

    def before_vpu(self, key, val, delay):
        self.due[1][key, self.now] = (self.now + delay, val)

    def tick(self, mxu):
        self.now += 1
        for w in (0, 1) if mxu else (1,):
            due = self.due[w]
            for key in [k for k, (t, _) in due.items() if t <= self.now]:
                self.slot[w] = (self.slot[w] + 1) % NZ
                self.put[w](self.slot[w], due.pop(key)[1])

    def zero(self):
        if self.z_ref is None:
            return jnp.zeros((8, 128), f32)
        return self.z_ref[0, pl.ds(0, 8), :]


K_MXU, K_ACC, K_SELF, K_SM0, K_SM1, K_FOLD, LAG = 6, 1, 3, 14, 8, 14, 4.5
M_STEPS = sum(5 + 24 + 3 + mt for mt in MT)
V_STEPS = sum(RT * (NT - mt) for mt in MT)


def _kernel(x_hbm, k_hbm, v_hbm, wq_hbm, wo_hbm, wg_hbm, wu_hbm, wd_hbm, o_ref,
            kb, vb, wq, wo, wg, wu, wd, q_s, s_s, p_s, pb_s, acc_s, z_s, e_s, xn_s, y_s, xb,
            sem_0, sem_p, sem_m):
    k_hbm, v_hbm, wq_hbm, wo_hbm = (r.bitcast(u32) for r in (k_hbm, v_hbm, wq_hbm, wo_hbm))

    def cp_kv(hbm, buf, p, sem):
        rows = pl.ds(p * (2 * RT), 2 * RT)
        return pltpu.make_async_copy(hbm.at[rows, pl.ds((SK - W) // 32, W // 32)], buf.at[rows], sem)

    def first_copies():
        sem = sem_0.at[0]
        return ([pltpu.make_async_copy(x_hbm, xb.at[:, pl.ds(0, D)], sem)]
                + [pltpu.make_async_copy(wq_hbm.at[:, pl.ds(128 * t, 128)], wq.at[t], sem)
                   for t in range(3 * NP)]
                + [cp_kv(k_hbm, kb, 0, sem)])

    def pair_copies(p, act):
        sem = sem_p.at[p % (LOOK + 1)]

        @pl.when(p + 1 < NP)
        def _():
            act(cp_kv(k_hbm, kb, p + 1, sem))

        act(cp_kv(v_hbm, vb, p, sem))
        rows = pl.ds(pl.multiple_of(p * DH, 64), DH)
        for c in range(5):
            act(pltpu.make_async_copy(wo_hbm.at[rows, pl.ds(128 * c, 128)], wo.at[p * 5 + c], sem))

    def glu_copies(j):
        if j == 0:
            return [pltpu.make_async_copy(a, b, sem_m.at[0]) for a, b in ((wg_hbm, wg), (wu_hbm, wu))]
        rows = pl.ds(CUTS[j - 1], CUTS[j] - CUTS[j - 1])
        return [pltpu.make_async_copy(wd_hbm.at[rows], wd.at[rows], sem_m.at[j])]

    for c in first_copies():
        c.start()
    for p in range(LOOK):
        pair_copies(p, lambda c: c.start())
    z_s[0, pl.ds(0, 8), :] = jnp.zeros((8, 128), f32)

    def project(p, pace, out):
        q = None
        for k in range(5):
            w = jnp.concatenate([_b(wq[3 * p + t, pl.ds(64 * k, 64), :]) for t in range(3)], axis=1)
            t = _dot(xn_s[:, pl.ds(128 * k, 128)] + pace.zero(), w)
            q = t if q is None else q + t
            pace.before_vpu(0, q[:, :128], K_MXU)
            yield
        out.append(q * _wide(xn_s[:, pl.ds(D, 128)], 3))

    def spread(q, a):
        lane = _iota(1)
        for g in range(12 * a, 12 * a + 12):
            qt = q[:, 128 * (g // 8):128 * (g // 8 + 1)]
            q_s[g] = jnp.take_along_axis(qt, ((lane >> 6) << 3) + (lane & 7) + 16 * (g % 8), axis=1)

    def scores(p, a, pace, consumed=lambda: True):
        diag = ((_iota(1) >> 3) & 7) == _iota(0)
        s = None
        for kt in range(12):
            lhs = jnp.where(diag, q_s[12 * a + kt], pace.zero())
            r0 = p * (2 * RT) + a * RT + 2 * kt
            rhs = jnp.concatenate(
                [_b(kb[pl.ds(r0, 2), pl.ds(32 * c, 32), :].reshape(64, 128)) for c in range(4)],
                axis=1)
            t = _dot(lhs, rhs)
            s = t if s is None else s + t
            pace.before_vpu(0, s[:, :128], K_MXU)
            yield
        assert consumed()
        if a == 1:
            s_s[...] = s
        else:
            p_s[...] = softmax_numerator(s, a, pace, K_SM0)

    def softmax_numerator(s, a, pace, delay):
        m = jnp.max(jnp.max(s, axis=1, keepdims=True), axis=0, keepdims=True)
        e = jnp.exp(s - m)
        pace.before_vpu(("sm", a), e[:, :128], delay)
        return e

    def row(pr, t):
        return jnp.broadcast_to(pr[t % 8:t % 8 + 1, 128 * (t // 8):128 * (t // 8 + 1)], (8, 128))

    def upper(p, rt, j):
        k = rt * NU + j
        return H * RT + 1 + p * (3 * NU) + k // 16, pl.ds(8 * (k % 16), 8), slice(None)

    def widen(p):
        for r in range(0, 2 * RT, 8):
            vs = {(rt, j): _b(vb[p * (2 * RT) + rt, pl.ds(8 * j, 8), :]).astype(f32)
                  for rt in range(r, r + 8) for j in range(NU)}
            for (rt, j), v in vs.items():
                vb[p * (2 * RT) + rt, pl.ds(8 * j, 8), :] = pltpu.bitcast(v[:8], u32)
                vb[upper(p, rt, j)] = pltpu.bitcast(v[8:], u32)

    def flip(p, mt):
        @pl.loop((NT - mt) // 2, NT // 2)
        def _(j):
            cols = pl.ds(pl.multiple_of(8 * j, 8), 8)
            vs = [_b(vb[pl.ds(p * (2 * RT) + 16 * u, 16), cols, :]).astype(f32) for u in range(3)]
            ts = [v[:, 8 * h:8 * h + 8, :].reshape(128, 128).T.astype(bf16)
                  for v in vs for h in range(2)]
            for n, t in enumerate(ts):
                vb[pl.ds(p * (2 * RT) + 8 * n, 8), cols, :] = (
                    pltpu.bitcast(t, u32).reshape(8, 8, 128))

    def pv_vpu(p, prs, pace, mt):
        nv = (NT - mt) // 2
        for a in range(2):
            e = [prs[a][:, 128 * c:128 * (c + 1)] for c in range(4)]
            e_s[:, pl.ds(384 + 128 * a, 128)] = (e[0] + e[1]) + (e[2] + e[3])
            have = []
            for r in range(a * RT, (a + 1) * RT, 6):
                acc = [None] * 6
                for n, i in [(n, i) for i0 in range(0, nv, 8) for n in range(6)
                             for i in range(i0, min(i0 + 8, nv))]:
                    j = (i + n) % nv
                    if j not in have:
                        have.append(j)
                        for t in (2 * j, 2 * j + 1):
                            pb_s[NT * a + t] = row(prs[a], t)
                    p0, p1 = pb_s[NT * a + 2 * j], pb_s[NT * a + 2 * j + 1]
                    v = vb[p * (2 * RT) + r + n, pl.ds(8 * j, 8), :]
                    if j < NU:
                        v0, v1 = pltpu.bitcast(v, f32), pltpu.bitcast(vb[upper(p, r + n, j)], f32)
                    else:
                        v = _b(v).astype(f32)
                        v0, v1 = v[:8], v[8:]
                    if acc[n] is None:
                        acc[n] = v0 * p0 + v1 * p1
                    else:
                        acc[n] = (acc[n] + v0 * p0) + v1 * p1
                    pace.before_mxu(r + n, acc[n], K_ACC)
                    if pace.now + K_SELF < K_MXU:
                        pace.before_vpu("self", acc[n], K_SELF)
                    yield
                for n in range(6):
                    acc_s[r + n] = acc[n]

    def pv_mxu(p, prs, pace, mt):
        o = None
        for t in range(NT - mt, NT):
            lhs = jnp.where(_iota(0) < 4, row(prs[0], t), row(prs[1], t)) + pace.zero()
            r0 = p * (2 * RT) + 8 * (t % 2)
            w = jnp.concatenate(
                [_b(vb[pl.ds(r0 + 16 * u, 8), pl.ds(8 * (t // 2), 8), :].reshape(64, 128))
                 for u in range(3)], axis=1)
            z = _dot(lhs, w)
            o = z if o is None else o + z
            pace.before_vpu(0, o[:, :128], K_MXU)
            yield
        e_s[:, pl.ds(0, 384)] = o

    def fold():
        def merge(lo, n):
            if n == 1:
                return jnp.broadcast_to(jnp.sum(acc_s[lo], axis=1, keepdims=True), (8, 128))
            n //= 2
            return jnp.where((_iota(1) & (8 * n)) == 0, merge(lo, n), merge(lo + n, n))

        tiles = [merge(16 * t, 16) for t in range(3)]
        inv = []
        for a in range(2):
            l = jnp.sum(e_s[:, pl.ds(384 + 128 * a, 128)], axis=0, keepdims=True)
            inv.append(jnp.broadcast_to(1.0 / jnp.sum(l, axis=1, keepdims=True), (8, 128)))
        inv = [inv[0], jnp.where(_iota(1) < 64, inv[0], inv[1]), inv[1]]
        return tiles, e_s[:, pl.ds(0, 384)], inv

    def out_project(p, o, pace, put):
        tiles, extra, inv = o
        y = None
        lane, sub = _iota(1), _iota(0)
        for t in range(3):
            w = jnp.concatenate([_b(wo[5 * p + c, pl.ds(64 * t, 64), :]) for c in range(5)], axis=1)
            lhs = jnp.where((lane & 7) == sub, tiles[t], pace.zero())
            pick = sub == (0, (lane >> 6) << 2, 4)[t]
            lhs = lhs + jnp.where(pick, extra[:, 128 * t:128 * (t + 1)], 0.0)
            z = _dot(lhs * inv[t], w)
            y = z if y is None else y + z
            pace.before_vpu(0, y[:, :128], K_MXU)
            yield
        put(y)

    def load(i):
        @pl.when(i + LOOK < NP)
        def _():
            pair_copies(i + LOOK, lambda c: c.start())

        @pl.when(i + LOOK == NP)
        def _():
            for j in range(len(CUTS)):
                for c in glu_copies(j):
                    c.start()

        pair_copies(i, lambda c: c.wait())
        flip(i, jnp.where((i & 1) == 0, MT[0], MT[1]))
        widen(i)

    def compute(n):
        off = n >> 8

        def to_mxu(slot, val):
            z_s[1 - off, pl.ds(8 * slot, 8), :] = val

        def to_vpu(slot, val):
            vb[H * RT - off, pl.ds(8 * slot, 8), :] = pltpu.bitcast(val, u32)

        pace = _Pace(to_mxu, to_vpu, z_s)
        prs, outs, scored = {}, {}, [0]

        def vpu_part(u):
            assert u in scored
            outs[u] = fold()
            prs[u] = [p_s[...], softmax_numerator(s_s[...], 1, pace, K_SM1)]
            for t in range(3):
                pace.before_vpu(("o", t), outs[u][0][t], K_FOLD + 2 * t)
            yield from pv_vpu(n * UNROLL + u, prs[u], pace, MT[u])

        def mxu_part(u):
            i = n * UNROLL + u

            def add(y):
                y_s[...] += y if u else jnp.where(i > 0, y, 0.0)

            q = []
            nxt = jnp.minimum(i + 1, NP - 1)
            yield from scores(nxt, 0, pace, lambda: u in prs)
            yield from project(jnp.minimum(i + 2, NP - 1), pace, q)
            spread(q[0], 0)
            yield from scores(nxt, 1, pace, lambda: u in prs)
            spread(q[0], 1)
            yield from pv_mxu(i, prs[u], pace, MT[u])
            yield from out_project(jnp.maximum(i - 1, 0), outs[u], pace, add)
            scored.append(u + 1)

        mxu = _chain(*[mxu_part(u) for u in range(UNROLL)])
        vpu = _chain(*[vpu_part(u) for u in range(UNROLL)])
        done = e = 0
        while done < V_STEPS:
            next(mxu, None)
            e += 1
            while done < min(V_STEPS, int(e * V_STEPS / (M_STEPS + LAG))):
                next(vpu, None)
                done += 1
            pace.tick(e < M_STEPS)
        _run(mxu, vpu)

    def finish(x, wait):
        y = []
        _run(out_project(NP - 1, fold(), _Pace(), y.append))
        x = x + jnp.sum(y_s[...] + y[0], axis=0, keepdims=True)
        d, r = _layernorm(x)
        h = []
        for cp in glu_copies(0) if wait else ():
            cp.wait()
        mean = jnp.sum(x, axis=-1, keepdims=True) * (1.0 / D)
        col = {k: jnp.broadcast_to(x[:1, k:k + 128], (128, 128)).T - mean[:1]
               for k in range(D - 128 * max(KV), D, 128)}
        for c, kv in zip(range(0, F, 256), KV):
            k0 = D - 128 * kv
            w = jnp.concatenate([m[pl.ds(0, k0), pl.ds(c, 256)] for m in (wg, wu)], axis=1)
            gu = _dot(d[:, :k0], w)
            if kv:
                acc = None
                for k in range(k0, D, 8):
                    w = jnp.concatenate(
                        [m[pl.ds(k, 8), pl.ds(c, 256)].astype(f32) for m in (wg, wu)], axis=1)
                    t = w * _wide(col[k // 128 * 128][k % 128:k % 128 + 8], 4)
                    acc = t if acc is None else acc + t
                gu = gu + jnp.sum(acc, axis=0, keepdims=True)
            gu = gu * _wide(r, 4)
            h.append((1.0 / (1.0 + jnp.exp(-gu[:, :256]))) * gu[:, 256:])
        h = jnp.concatenate(h, axis=1)
        for j, (lo, hi) in enumerate(zip(CUTS, CUTS[1:])):
            for cp in glu_copies(1 + j) if wait else ():
                cp.wait()
            x = x + _dot(h[:, lo:hi], wd[pl.ds(lo, hi - lo), :])
        return x

    def layer(li, x):
        d, r = _layernorm(x)
        xn_s[:, pl.ds(0, D)] = d
        xn_s[:, pl.ds(D, 128)] = r * (DH ** -0.5)

        free = _Pace()
        q = []
        _run(project(0, free, q))
        spread(q[0], 0)
        spread(q[0], 1)
        _run(project(1, free, q), scores(0, 0, free), scores(0, 1, free))
        spread(q[1], 0)
        spread(q[1], 1)
        acc_s[...] = jnp.zeros(acc_s.shape, f32)
        e_s[...] = jnp.ones(e_s.shape, f32)
        y_s[...] = jnp.zeros(y_s.shape, f32)

        def step(n, carry):
            @pl.loop(li * UNROLL, UNROLL)
            def _(u):
                load(n * UNROLL + u)

            compute(n)
            return carry

        lax.fori_loop(0, NP // UNROLL, step, 0)
        return lax.cond(li == 0, lambda x: finish(x, True), lambda x: finish(x, False), x)

    for c in first_copies():
        c.wait()
    x0 = jnp.broadcast_to(xb[:, pl.ds(0, D)].astype(f32), (8, D))
    x = lax.fori_loop(0, LAYERS, layer, x0)
    o_ref[...] = x[:1].astype(o_ref.dtype)


@jax.jit
def pallas_interleave_layers__sliding_block_cached__glu_gated_glu__decode_kernel(
    A_x: jax.Array,
    A_k_cache: jax.Array,
    A_v_cache: jax.Array,
    A_wq: jax.Array,
    A_wo: jax.Array,
    B_x: jax.Array,
    B_w_gate: jax.Array,
    B_w_up: jax.Array,
    B_w_down: jax.Array,
):
    del B_x
    assert A_k_cache.shape == A_v_cache.shape == (1, H, SK, DH)
    kt = _tiles(jnp.swapaxes(A_k_cache, 2, 3).reshape(H * DH, SK))
    vt = _tiles(jnp.swapaxes(A_v_cache, 2, 3).reshape(H * DH, SK))
    out = pl.pallas_call(
        _kernel,
        out_shape=jax.ShapeDtypeStruct((1, D), A_x.dtype),
        in_specs=[pl.BlockSpec(memory_space=pltpu.HBM)] * 8,
        out_specs=pl.BlockSpec(memory_space=pltpu.VMEM),
        scratch_shapes=[
            pltpu.VMEM((H * RT, W // 32, 128), u32),
            pltpu.VMEM((H * RT + 1 + NP * 3 * NU, W // 32, 128), u32),
            pltpu.VMEM((3 * NP, D // 2, 128), u32),
            pltpu.VMEM((5 * NP, DH, 128), u32),
            pltpu.VMEM((D, F), bf16),
            pltpu.VMEM((D, F), bf16),
            pltpu.VMEM((F, D), bf16),
            pltpu.VMEM((24, 8, 128), f32),
            pltpu.VMEM((8, 512), f32),
            pltpu.VMEM((8, 512), f32),
            pltpu.VMEM((2 * NT, 8, 128), f32),
            pltpu.VMEM((2 * RT, 8, 128), f32),
            pltpu.VMEM((2, NZ * 8, 128), f32),
            pltpu.VMEM((8, 1024), f32),
            pltpu.VMEM((8, D + 384), f32),
            pltpu.VMEM((8, D), f32),
            pltpu.VMEM((1, 2 * D), bf16),
            pltpu.SemaphoreType.DMA((1,)),
            pltpu.SemaphoreType.DMA((LOOK + 1,)),
            pltpu.SemaphoreType.DMA((len(CUTS),)),
        ],
        compiler_params=pltpu.CompilerParams(vmem_limit_bytes=127 * 1024 * 1024),
    )(A_x.reshape(1, D), kt, vt, A_wq, A_wo, B_w_gate, B_w_up, B_w_down)
    return out.reshape(1, 1, D)
```
